```python
import jax
import jax.numpy as jnp

def _softmax(x, axis=-1):
    return jax.nn.softmax(x, axis=axis)
def _gelu(x):
    return jax.nn.gelu(x, approximate=True)
def _silu(x):
    return jax.nn.silu(x)
def _sigmoid(x):
    return jax.nn.sigmoid(x)
def _layernorm(x, axis=-1, eps=1e-5):
    m = jnp.mean(x, axis=axis, keepdims=True)
    v = jnp.var(x, axis=axis, keepdims=True)
    return (x - m) / jnp.sqrt(v + eps)
def _scatter_add(tgt, idx, src, axis=0):
    return tgt.at[idx].add(src)
def _segment_sum(src, seg, n):
    return jax.ops.segment_sum(src, seg, n)
class _Rng:
    def __init__(self, key):
        self._k = key
    def _next(self):
        self._k, sub = jax.random.split(self._k)
        return sub
    def normal(self, shape):
        return jax.random.normal(self._next(), shape, dtype=jnp.bfloat16)
    def randint(self, lo, hi, shape):
        return jax.random.randint(self._next(), shape, lo, hi, dtype=jnp.int32)
    def uniform(self, shape, lo=0.0, hi=1.0):
        return jax.random.uniform(self._next(), shape, jnp.bfloat16, lo, hi)
    def permutation(self, n):
        return jax.random.permutation(self._next(), n)


kernel_name = 'interleave_layers__gqa_block_cached__sliding_block_cached__decode'

def _fwd_setup_inputs():
    _rng = _Rng(jax.random.key(int.from_bytes(__import__("os").urandom(4), "little")))
    _w = (lambda a: (lambda t: t.astype(jnp.bfloat16) if jnp.issubdtype(t.dtype, jnp.floating) else t)(jnp.asarray(a)))
    def _A_setup():
        B, Sq, D = 1, 1, 640
        Hq, Hkv, Sk, Dh = 32, 32, 8192, 128
        assert Hq % Hkv == 0, (Hq, Hkv)
        return {
            "x": _w((lambda *s: _rng.normal(s) * 0.05)(B, Sq, D)),
            "k_cache": _w((lambda *s: _rng.normal(s) * 0.05)(B, Hkv, Sk, Dh)),
            "v_cache": _w((lambda *s: _rng.normal(s) * 0.05)(B, Hkv, Sk, Dh)),
            "wq": _w((lambda *s: _rng.normal(s) * 0.05)(D, Hq * Dh) * (D ** -0.5)),
            "wo": _w((lambda *s: _rng.normal(s) * 0.05)(Hq * Dh, D) * ((Hq * Dh) ** -0.5)),
        }
    _A_in = _A_setup()

    def _B_setup():
        B, Sq, D = 1, 1, 640
        Hq, Hkv, Sk, Dh = 32, 32, 8192, 128
        assert Hq % Hkv == 0, (Hq, Hkv)
        return {
            "x": _w((lambda *s: _rng.normal(s) * 0.05)(B, Sq, D)),
            "k_cache": _w((lambda *s: _rng.normal(s) * 0.05)(B, Hkv, Sk, Dh)),
            "v_cache": _w((lambda *s: _rng.normal(s) * 0.05)(B, Hkv, Sk, Dh)),
            "wq": _w((lambda *s: _rng.normal(s) * 0.05)(D, Hq * Dh) * (D ** -0.5)),
            "wo": _w((lambda *s: _rng.normal(s) * 0.05)(Hq * Dh, D) * ((Hq * Dh) ** -0.5)),
        }
    _B_in = _B_setup()

    return {
        "A_x": _A_in["x"],
        "A_k_cache": _A_in["k_cache"],
        "A_v_cache": _A_in["v_cache"],
        "A_wq": _A_in["wq"],
        "A_wo": _A_in["wo"],
        "B_x": _B_in["x"],
        "B_k_cache": _B_in["k_cache"],
        "B_v_cache": _B_in["v_cache"],
        "B_wq": _B_in["wq"],
        "B_wo": _B_in["wo"],
    }

def _fwd_reference(A_x, A_k_cache, A_v_cache, A_wq, A_wo, B_x, B_k_cache, B_v_cache, B_wq, B_wo):
    def _A_ref(x, k_cache, v_cache, wq, wo):
        B, Sq, D = x.shape
        Hq, Dh = 32, 128
        Hkv = k_cache.shape[1]
        rep = Hq // Hkv
        q = (lambda x, *d: x.transpose(*d))((x @ wq).reshape(B, Sq, Hq, Dh), 0, 2, 1, 3)
        k = jnp.repeat(k_cache, rep, axis=1)
        v = jnp.repeat(v_cache, rep, axis=1)
        scores = jnp.einsum("bhqd,bhkd->bhqk", q, k) * (Dh ** -0.5)
        p = _softmax(scores, axis=-1)
        o = jnp.einsum("bhqk,bhkd->bhqd", p, v)
        return (lambda x, *d: x.transpose(*d))(o, 0, 2, 1, 3).reshape(B, Sq, Hq * Dh) @ wo

    def _B_ref(x, k_cache, v_cache, wq, wo):
        B, Sq, D = x.shape
        Hq, Dh = 32, 128
        Hkv, Sk = k_cache.shape[1], k_cache.shape[2]
        W = min(4096, max(256, Sk // 4))
        rep = Hq // Hkv
        q = (lambda x, *d: x.transpose(*d))((x @ wq).reshape(B, Sq, Hq, Dh), 0, 2, 1, 3)
        k = jnp.repeat(k_cache[:, :, Sk - W:, :], rep, axis=1)
        v = jnp.repeat(v_cache[:, :, Sk - W:, :], rep, axis=1)
        scores = jnp.einsum("bhqd,bhkd->bhqk", q, k) * (Dh ** -0.5)
        p = _softmax(scores, axis=-1)
        o = jnp.einsum("bhqk,bhkd->bhqd", p, v)
        return (lambda x, *d: x.transpose(*d))(o, 0, 2, 1, 3).reshape(B, Sq, Hq * Dh) @ wo

    x = A_x
    x = x + _A_ref(_layernorm(x, axis=-1), A_k_cache, A_v_cache, A_wq, A_wo)
    x = x + _B_ref(_layernorm(x, axis=-1), B_k_cache, B_v_cache, B_wq, B_wo)
    x = x + _A_ref(_layernorm(x, axis=-1), A_k_cache, A_v_cache, A_wq, A_wo)
    x = x + _B_ref(_layernorm(x, axis=-1), B_k_cache, B_v_cache, B_wq, B_wo)
    return x


def setup_inputs():
    _inp = _fwd_setup_inputs()
    _gk = jax.random.fold_in(jax.random.key(int.from_bytes(__import__("os").urandom(4), "little")), 2**31 - 1)
    _shapes = [[1, 1, 640]]
    _dtypes = ['bfloat16']
    _gks = jax.random.split(_gk, len(_shapes))
    _gs = [jax.random.normal(k, s, dtype=jnp.dtype(d)) * 0.05 for k, s, d in zip(_gks, _shapes, _dtypes)]
    _inp["grad_out"] = _gs[0]
    return _inp

def reference(A_x, A_k_cache, A_v_cache, A_wq, A_wo, B_k_cache, B_v_cache, B_wq, B_wo, B_x, grad_out):
    _const = dict(B_x=B_x)
    def _f(*_d):
        return _fwd_reference(**{'A_x': _d[0], 'A_k_cache': _d[1], 'A_v_cache': _d[2], 'A_wq': _d[3], 'A_wo': _d[4], 'B_k_cache': _d[5], 'B_v_cache': _d[6], 'B_wq': _d[7], 'B_wo': _d[8], **_const})
    _out, _vjp = jax.vjp(_f, A_x, A_k_cache, A_v_cache, A_wq, A_wo, B_k_cache, B_v_cache, B_wq, B_wo)
    _grads = _vjp(grad_out)
    _out0 = jnp.asarray(_out)
    return (_out0, *[jnp.asarray(_g) for _g in _grads])
```

```python
import jax
from jax import lax
import jax.numpy as jnp
import jax.experimental.pallas as pl
import jax.experimental.pallas.tpu as pltpu

D = 640
H = 32
DH = 128
QR = 2048
S = 4 * QR
BR = 512
NB = 4 * H
NS = 16
KEEP = NS // 4
EPS = 1e-5
SCALE = DH ** -0.5

ZN = 192
Z_BUBBLE = 2

F32 = jnp.float32
BF16 = jnp.bfloat16
U32 = jnp.uint32
NT = (((1,), (1,)), ((), ()))


def _mo(i, n):
    return i if isinstance(i, int) else pl.multiple_of(i, n)


def _dot(a, b):
    return jnp.dot(a, b, preferred_element_type=F32)


def _dot_nt(a, b):
    return lax.dot_general(a, b, NT, preferred_element_type=F32)


def _iota(shape, axis):
    return lax.broadcasted_iota(jnp.int32, shape, axis)


def _layernorm(x):
    xc = x - jnp.mean(x, axis=1, keepdims=True)
    sigma = jnp.sqrt(jnp.mean(xc * xc, axis=1, keepdims=True) + EPS)
    return xc / sigma, sigma


def _layernorm_bwd(dn, n, sigma):
    m1 = jnp.mean(dn, axis=1, keepdims=True)
    m2 = jnp.mean(dn * n, axis=1, keepdims=True)
    return (dn - m1 - n * m2) / sigma


def _kernel(
        x_h, g_h, ka_h, va_h, wqa_h, woa_h, kb_h, vb_h, wqb_h, wob_h,
        out_h, dx_h, dka_h, dva_h, dwqa_h, dwoa_h, dkb_h, dvb_h, dwqb_h, dwob_h,
        va, kb, vb, wqa, woa, wqb, wob, ring, j1, s_scr, ra, rb, oa, ob,
        dqa, dqb, kbar, inv, zero, x_v, g_v, out_v, dx_v,
        ksem, vsem, bsem, wsem, ssem, zsem, osem):
    ring32 = ring.bitcast(U32)
    ringf = ring.bitcast(F32)
    va32 = va.bitcast(U32)
    kb32 = kb.bitcast(U32)
    vb32 = vb.bitcast(U32)

    def wait_all(buf, sem):
        pltpu.make_async_copy(buf, buf, sem).wait()

    def k_copy(head, c, slot, i):
        src = ka_h.at[head, :, pl.ds(_mo(c * BR + i * 32, 32), 32), :]
        return pltpu.make_async_copy(
            src, ring.at[slot, :, pl.ds(i * 32, 32), :], ksem.at[slot])

    def k_start(head, c, slot):
        for i in range(BR // 32):
            k_copy(head, c, slot, i).start(priority=i % 2)

    def k_wait(slot):
        wait_all(ring.at[slot], ksem.at[slot])

    def v_copy(grp, q, r):
        sl = (pl.ds(4 * grp, 4), q, pl.ds(_mo(r, 32), 32))
        return pltpu.make_async_copy(va_h.at[sl], va.at[sl], vsem.at[grp])

    def b_start(grp, i):
        heads, r = pl.ds(4 * grp, 4), pl.ds(_mo(i * 32, 32), 32)
        pltpu.make_async_copy(
            kb_h.at[heads, 3, r], kb.at[heads, r], bsem.at[0, grp]).start(priority=0)
        pltpu.make_async_copy(
            vb_h.at[heads, 3, r], vb.at[heads, r], bsem.at[1, grp]).start(priority=1)

    def wq_start(src, dst, sem, i):
        for u in range(8):
            sl = (slice(None), pl.ds(_mo(i * 8, 8), 8), pl.ds(u * 512, 512))
            pltpu.make_async_copy(src.at[sl], dst.at[sl], sem).start(priority=u % 2)

    def wo_start(src, dst, sem, i):
        for u in range(8):
            sl = (pl.ds((u % 2) * 4, 4), pl.ds(_mo(i * 32 + (u // 2) * 8, 8), 8))
            pltpu.make_async_copy(src.at[sl], dst.at[sl], sem).start(priority=u % 2)

    def zero_start(which, z):
        dst = (dkb_h, dvb_h)[which].at[
            pl.ds((z // 48) * 8, 8), (z % 48) // 16, pl.ds(_mo((z % 16) * 128, 128), 128)]
        pltpu.make_async_copy(zero, dst, zsem.at[which]).start()

    def zero_range(which, lo, hi):
        lax.fori_loop(lo, hi, lambda z, _: zero_start(which, z), None)

    def dwq_start(src, dst, sem, i):
        sl = (slice(None), pl.ds(_mo((i // 2) * 8, 8), 8), pl.ds(_mo((i % 2) * 2048, 2048), 2048))
        pltpu.make_async_copy(src.at[sl], dst.at[sl], sem).start()

    def dwo_start(src, dst, sem, i):
        sl = (slice(None), pl.ds(_mo(i * 16, 16), 16))
        pltpu.make_async_copy(src.at[sl], dst.at[sl], sem).start()

    def to_heads(blocks):
        row = _iota((8, DH), 0)
        acc = blocks[0]
        for u in range(1, 8):
            acc = jnp.where(row == u, blocks[u], acc)
        return acc

    def to_flat(ref, r):
        return jnp.concatenate(
            [jnp.broadcast_to(ref[pl.ds(r + u, 1), :], (8, DH)) for u in range(4)], axis=1)

    def lanes(a):
        return [a[:, u * DH:(u + 1) * DH] for u in range(a.shape[1] // DH)]

    def q_proj(n, wq, dst, r):
        n = n.astype(BF16)

        def body(grp, _):
            cols = pl.ds(_mo(grp * 1024, 1024), 1024)
            acc = sum(_dot(n[:, k * 128:(k + 1) * 128], wq[k, :, cols]) for k in range(D // 128))
            dst[pl.ds(_mo(r + grp * 8, 8), 8), :] = to_heads(lanes(acc))
        lax.fori_loop(0, H // 8, body, None)

    def q_proj_bwd(src, r, wq):
        def body(i, acc):
            dq = to_flat(src, r + 4 * i).astype(BF16)
            cols = pl.ds(_mo(i * 512, 512), 512)
            return acc + jnp.concatenate(
                [_dot_nt(dq, wq[k, :, cols]) for k in range(D // 128)], axis=1)
        return lax.fori_loop(0, H // 4, body, jnp.zeros((8, D), F32), unroll=2)

    def o_proj(src, r, wo):
        def body(i, acc):
            return acc + _dot(to_flat(src, r + 4 * i).astype(BF16), wo[i])
        return lax.fori_loop(0, H // 4, body, jnp.zeros((8, D), F32), unroll=2)

    def o_proj_bwd(g, wo, dst, r):
        g = g.astype(BF16)

        def body(grp, _):
            do = lanes(_dot_nt(g, wo[2 * grp])) + lanes(_dot_nt(g, wo[2 * grp + 1]))
            dst[pl.ds(_mo(r + grp * 8, 8), 8), :] = to_heads(do)
        lax.fori_loop(0, H // 8, body, None)

    def row8(ref, r):
        return jnp.broadcast_to(ref[pl.ds(r, 1), :], (8, DH))

    def pair8(ref, r_even, r_odd):
        return jnp.where(_iota((8, DH), 0) % 2 == 0, row8(ref, r_even), row8(ref, r_odd))

    ninf = jnp.full((8, DH), -jnp.inf, F32)

    def a_query(head, second):
        q = pair8(ra, head, H + head) if second else row8(ra, head)
        return q.astype(BF16)

    def j3_at(head):
        return (head // 8, 2 + (head % 8) // 4, pl.ds(_mo((head % 4) * 64, 64), 64))

    def a_scores(q, c, qq, slot, mx):
        s = _dot_nt(q, pltpu.bitcast(ring32[slot, qq], BF16)) * SCALE
        s_scr[:, pl.ds((c * 4 + qq) * BR, BR)] = s
        for tile in lanes(s):
            mx = jnp.maximum(mx, tile)
        return mx

    def a_accumulate(head, c, qq, slot, m, carry, second):
        acc, ksum, l = carry
        e = jnp.exp(s_scr[:, pl.ds((c * 4 + qq) * BR, BR)] - m)
        for tile in lanes(e):
            l = l + tile
        e2 = jnp.concatenate([e, e], axis=0).astype(BF16)
        if second:
            e = jnp.broadcast_to(e[1:2], (8, BR))
        for u in range(BR // DH):
            k = pltpu.bitcast(ring32[slot, qq, pl.ds(u * DH // 2, DH // 2), :], BF16)
            v = pltpu.bitcast(va32[head, qq, pl.ds((c * BR + u * DH) // 2, DH // 2), :], BF16)
            w = k.T.astype(F32).reshape(DH // 8, 8, DH) * lanes(e)[u][None]
            w = jnp.concatenate([w.reshape(DH, DH).astype(BF16), lanes(e2)[u]], axis=0)
            acc = acc + _dot(w, v)
        ksum = ksum + _dot(e2, pltpu.bitcast(ring32[slot, qq], BF16))[:8]
        return (acc, ksum, l), lanes(pltpu.bitcast(e2, U32))

    def a_head(head, slot, nxt, nxt_slot, m, second, issue):
        carry = (jnp.zeros((DH + 16, DH), F32), jnp.zeros((8, DH), F32),
                 jnp.zeros((8, DH), F32))
        mx = ninf
        q = a_query(nxt, second)
        pairs = []
        for c in range(4):
            for qq in range(4):
                carry, e_tiles = a_accumulate(head, c, qq, slot + c, m, carry, second)
                pairs += e_tiles
                mx = a_scores(q, c, qq, nxt_slot + c, mx)
            issue(c)
        acc, ksum, l = carry
        rl = jnp.broadcast_to(1.0 / jnp.sum(l, axis=1, keepdims=True), (8, DH))
        row = pl.ds(H + head if second else head, 1)
        kpv = (acc[:DH] * rl[1:2]).astype(BF16)
        oa[row, :] = acc[DH + 1:DH + 2] * rl[1:2]
        kbar[row, :] = ksum[1:2] * rl[1:2]
        if second:
            ring32[j3_at(head)] = pltpu.bitcast(kpv, U32)
            for i in range(8):
                ring32[i // 2, i % 2, pl.ds(_mo(head * 8, 8), 8), :] = (
                    to_heads(pairs[8 * i:8 * i + 8]))
            inv[pl.ds(head, 1), :] = rl[0:1]
            inv[row, :] = rl[1:2]
        else:
            j1[head] = kpv
        return jnp.max(mx, axis=1, keepdims=True)

    def a_first_scores(head, slot, second):
        mx = ninf
        q = a_query(head, second)
        for c in range(4):
            for qq in range(4):
                mx = a_scores(q, c, qq, slot + c, mx)
        return jnp.max(mx, axis=1, keepdims=True)

    def a_delta(r, n):
        do = ra[pl.ds(2 * H + r, n), :].astype(BF16).astype(F32)
        return jnp.sum(do * oa[pl.ds(r, n), :], axis=1, keepdims=True)

    def a_dq(kpv, r):
        def body(head, _):
            do = row8(ra, 2 * H + r + head).astype(BF16)
            dqa[pl.ds(r + head, 1), :] = _dot_nt(do, kpv(head))[0:1]
        lax.fori_loop(0, H, body, None, unroll=4)
        rows = pl.ds(r, H)
        dqa[rows, :] = (dqa[rows, :] - kbar[rows, :] * a_delta(r, H)) * SCALE

    def b_softmax(q, k):
        s = _dot_nt(q.astype(BF16), k) * SCALE
        e = jnp.exp(s - jnp.max(s, axis=1, keepdims=True))
        return e * (1.0 / jnp.sum(e, axis=1, keepdims=True))

    def b_ds(p, do, v):
        dp = _dot_nt(do.astype(BF16), v)
        return p * (dp - jnp.sum(p * dp, axis=1, keepdims=True)) * SCALE

    def wb_at(t, r, n):
        return (4 + t // 8, (t % 8) // 2, pl.ds((t % 2) * 128 + r, n))

    def wb_store(r, val):
        for t in range(QR // DH):
            ringf[wb_at(t, r, 1)] = val[:, t * DH:(t + 1) * DH]

    def dp_at(t, r, n):
        return (8 + t // 16, (t % 16) // 4, pl.ds(_mo((t % 4) * 64, 64) + r, n))

    def select_head(r_ref, head, lo):
        row = _iota((4 * H, DH), 0)
        keep = (row == lo + head) | (row == lo + H + head)
        return jnp.where(keep, r_ref[...], 0.0).astype(BF16)

    def weight_grads(wq, wo, dq, o, n_a, n_b, g_a, g_b, issue):
        row = _iota((DH, D), 0)
        nt = jnp.where(row == 0, n_a[0:1], jnp.where(row == 1, n_b[0:1], 0.0))
        nt = nt.T.astype(BF16)
        ot = jnp.concatenate([o[...], jnp.zeros((2 * H, DH), F32)], axis=0)
        ot = ot.T.astype(BF16)

        def body(head, _):
            r = _iota((DH, DH), 0)
            sel = jnp.where(r == 0, dq[pl.ds(head, 1), :],
                            jnp.where(r == 1, dq[pl.ds(H + head, 1), :], 0.0))
            dwq = _dot(nt, sel.astype(BF16)).astype(BF16)
            wq[:, :, pl.ds(_mo(head * DH, DH), DH)] = dwq.reshape(D // DH, DH, DH)
            sel = jnp.where(row == head, g_a[0:1],
                            jnp.where(row == H + head, g_b[0:1], 0.0))
            dwo = _dot(ot, sel.astype(BF16)).astype(BF16)
            wo[head // 4, pl.ds(_mo((head % 4) * DH, DH), DH), :] = dwo
            issue(head)
        lax.fori_loop(0, H, body, None)

    x_copy = pltpu.make_async_copy(x_h, x_v, ssem.at[0])
    g_copy = pltpu.make_async_copy(g_h, g_v, ssem.at[1])
    x_copy.start()
    g_copy.start()
    lax.fori_loop(0, 16, lambda i, _: wq_start(wqa_h, wqa, wsem.at[0], i), None)
    first = H - KEEP

    def l1_slot(h):
        return 4 * ((h + KEEP - first % KEEP) % KEEP)
    lax.fori_loop(0, 8, lambda b, _: k_start(b // 4, b % 4, l1_slot(b // 4) + b % 4), None)
    zero[...] = jnp.zeros(zero.shape, BF16)
    x_copy.wait()
    g_copy.wait()
    x0 = jnp.broadcast_to(x_v[0].astype(F32), (8, D))
    g4 = jnp.broadcast_to(g_v[0].astype(F32), (8, D))
    n1, sigma1 = _layernorm(x0)
    wait_all(wqa, wsem.at[0])
    q_proj(n1, wqa, ra, 0)

    def first_group(i, _):
        for u in range(8):
            v_copy(0, i // 8, (i % 8) * 256 + u * 32).start(priority=u % 2)
    lax.fori_loop(0, 32, first_group, None)
    for c in range(4):
        k_wait(l1_slot(0) + c)
    m = a_first_scores(0, l1_slot(0), False)
    lax.fori_loop(8, 16, lambda b, _: k_start(b // 4, b % 4, l1_slot(b // 4) + b % 4), None)

    def l1_wait(h):
        @pl.when(h % 4 == 0)
        def _():
            wait_all(va.at[pl.ds(0, 4)], vsem.at[h // 4])

    def l1_stream(h, m):
        l1_wait(h)
        for c in range(4):
            k_wait(l1_slot(h + 1) + c)
        slot = l1_slot(h + 4)

        def issue(c):
            for i in range(BR // 32):
                k_copy(h + 4, c, slot + c, i).start(priority=0)
                v_copy(h // 4 + 1, h % 4, c * BR + i * 32).start(priority=1)
        return a_head(h, l1_slot(h), h + 1, l1_slot(h + 1), m, False, issue)
    m = lax.fori_loop(0, H - 4, l1_stream, m)

    def l1_tail(h, m):
        l1_wait(h)
        nxt = jnp.minimum(h + 1, H - 1)

        @pl.when(h + 1 < H)
        def _():
            for c in range(4):
                k_wait(l1_slot(nxt) + c)

        def issue(c):
            i = (h - (H - 4)) * 4 + c
            wo_start(woa_h, woa, wsem.at[1], i)
            wq_start(wqb_h, wqb, wsem.at[2], i)
            for u in range(4):
                b_start(0, i * 4 + u)
        return a_head(h, l1_slot(h), nxt, l1_slot(nxt), m, False, issue)
    lax.fori_loop(H - 4, H, l1_tail, m)

    lax.fori_loop(0, 32, lambda i, _: b_start(1, i), None)
    wait_all(woa, wsem.at[1])
    x1 = x0 + o_proj(oa, 0, woa)
    n2, sigma2 = _layernorm(x1)
    lax.fori_loop(32, 64, lambda i, _: b_start(1, i), None)
    wait_all(wqb, wsem.at[2])
    q_proj(n2, wqb, rb, 0)

    def l2_head(h, _):
        @pl.when(h % 4 == 0)
        def _():
            wait_all(kb.at[pl.ds(0, 4)], bsem.at[0, h // 4])
            wait_all(vb.at[pl.ds(0, 4)], bsem.at[1, h // 4])

        @pl.when(h < H - 8)
        def _():
            for u in range(16):
                b_start(h // 4 + 2, (h % 4) * 16 + u)

        @pl.when((h >= H - 8) & (h < H - 4))
        def _():
            for u in range(4):
                wo_start(wob_h, wob, wsem.at[3], (h - (H - 8)) * 4 + u)

        @pl.when(h >= H - 4)
        def _():
            for u in range(2 * Z_BUBBLE):
                zero_start(0, (h - (H - 4)) * 2 * Z_BUBBLE + u)
        p = b_softmax(row8(rb, h), pltpu.bitcast(kb32[h], BF16))
        ob[pl.ds(h, 1), :] = _dot(p.astype(BF16), pltpu.bitcast(vb32[h], BF16))[0:1]
    lax.fori_loop(0, H, l2_head, None)
    wait_all(wob, wsem.at[3])
    x2 = x1 + o_proj(ob, 0, wob)

    n3, sigma3 = _layernorm(x2)
    q_proj(n3, wqa, ra, H)
    m = a_first_scores(first, 0, True)
    z0 = 8 * Z_BUBBLE
    z1 = z0 + 56

    def l3_slot(j):
        return jnp.where(j == 0, 0, 4 + 4 * ((j + KEEP - 2) % (KEEP - 1)))

    def l3_head(j, m, issue):
        nxt = jnp.minimum(j + 1, H - 1)

        @pl.when((j + 1 >= KEEP) & (j + 1 < H))
        def _():
            for c in range(4):
                k_wait(l3_slot(nxt) + c)
        return a_head((first + j) % H, l3_slot(j), (first + nxt) % H, l3_slot(nxt),
                      m, True, issue)

    def l3_stream(j, m):
        slot = l3_slot(j)
        return l3_head(j, m, lambda c: k_start(j - 1, c, slot + c))

    def l3_quiet(j, m):
        @pl.when(j == first + 2)
        def _():
            zero_range(0, z0, z1)
        return l3_head(j, m, lambda c: None)

    def l3_part(part, m):
        lo = jnp.where(part == 0, 0, first + 1)
        mid = jnp.where(part == 0, 1, H)
        hi = jnp.where(part == 0, first + 1, H)
        return lax.fori_loop(mid, hi, l3_stream, lax.fori_loop(lo, mid, l3_quiet, m))
    lax.fori_loop(0, 2, l3_part, m)
    x3 = x2 + o_proj(oa, H, woa)

    n4, sigma4 = _layernorm(x3)
    q_proj(n4, wqb, rb, H)
    o_proj_bwd(g4, wob, rb, 3 * H)

    def l4_head(h, _):
        for u in range(3):
            zero_start(0, z1 + 3 * h + u)
        k = pltpu.bitcast(kb32[h], BF16)
        v = pltpu.bitcast(vb32[h], BF16)
        p = b_softmax(pair8(rb, h, H + h), k)
        ob[pl.ds(H + h, 1), :] = _dot(p.astype(BF16), v)[1:2]
        ds = b_ds(p, row8(rb, 3 * H + h), v)
        dqb[pl.ds(H + h, 1), :] = _dot(ds.astype(BF16), k)[1:2]
        wb_store(H + h, ds[1:2])
        wb_store(2 * H + h, p[0:1])
        wb_store(3 * H + h, p[1:2])
    lax.fori_loop(0, H, l4_head, None)
    zero_range(0, z1 + 3 * H, ZN)
    zero_range(1, 0, 16)

    out_v[0] = (x3 + o_proj(ob, H, wob))[0:1].astype(BF16)
    out_copy = pltpu.make_async_copy(out_v, out_h, ssem.at[2])
    out_copy.start()
    g3 = g4 + _layernorm_bwd(q_proj_bwd(dqb, H, wqb), n4, sigma4)

    o_proj_bwd(g3, woa, ra, 3 * H)
    a_dq(lambda head: pltpu.bitcast(ring32[j3_at(head)], BF16), H)
    g2 = g3 + _layernorm_bwd(q_proj_bwd(dqa, H, wqa), n3, sigma3)

    o_proj_bwd(g2, wob, rb, 2 * H)

    def l2_bwd_head(h, _):
        for u in range(3):
            zero_start(1, 16 + 3 * h + u)
        p = jnp.concatenate(
            [jnp.broadcast_to(ringf[wb_at(t, 2 * H + h, 1)], (8, DH))
             for t in range(QR // DH)], axis=1)
        ds = b_ds(p, row8(rb, 2 * H + h), pltpu.bitcast(vb32[h], BF16))
        dqb[pl.ds(h, 1), :] = _dot(ds.astype(BF16), pltpu.bitcast(kb32[h], BF16))[0:1]
        wb_store(h, ds[0:1])
    lax.fori_loop(0, H, l2_bwd_head, None)
    zero_range(1, 16 + 3 * H, ZN - H)
    g1 = g2 + _layernorm_bwd(q_proj_bwd(dqb, 0, wqb), n2, sigma2)

    o_proj_bwd(g1, woa, ra, 2 * H)
    a_dq(lambda head: j1[head], 0)
    g0 = g1 + _layernorm_bwd(q_proj_bwd(dqa, 0, wqa), n1, sigma1)
    dx_v[0] = g0[0:1].astype(BF16)
    dx_copy = pltpu.make_async_copy(dx_v, dx_h, ssem.at[3])
    dx_copy.start()

    for t in range(QR // DH):
        tile = ringf[wb_at(t, 0, 4 * H)].T.astype(BF16)
        ring32[6, t // 4, pl.ds((t % 4) * 64, 64), :] = pltpu.bitcast(tile, U32)

    def b_grad_start(src, dst, sem, i):
        heads, r = pl.ds((i // 16) * 8, 8), pl.ds(_mo((i % 16) * 128, 128), 128)
        pltpu.make_async_copy(src.at[heads, r], dst.at[heads, 3, r], sem).start()

    def b_grads(grp, _):
        for u in range(8):
            head = grp * 8 + u
            for dst, lo in ((vb32, 2 * H), (kb32, 0)):
                sel = select_head(rb, head, lo)
                for qq in range(4):
                    val = _dot(pltpu.bitcast(ring32[6, qq], BF16), sel).astype(BF16)
                    dst[head, pl.ds(qq * BR // 2, BR // 2), :] = pltpu.bitcast(val, U32)
        for i in range(16):
            b_grad_start(vb, dvb_h, osem.at[0], grp * 16 + i)
    lax.fori_loop(0, 4, b_grads, None)

    weight_grads(wqb, wob, dqb, ob, n2, n4, g2, g4,
                 lambda head: b_grad_start(kb, dkb_h, osem.at[1], head))
    weight_grads(wqa, woa, dqa, oa, n1, n3, g1, g3,
                 lambda head: b_grad_start(kb, dkb_h, osem.at[1], H + head))

    def a_dp(h, _):
        zero_start(1, ZN - H + h)
        dwq_start(wqb, dwqb_h, osem.at[2], h)
        dwo_start(wob, dwob_h, osem.at[3], h)
        dwq_start(wqa, dwqa_h, osem.at[4], h)
        dwo_start(woa, dwoa_h, osem.at[5], h)
        do = pair8(ra, 2 * H + h, 3 * H + h).astype(BF16)
        for qq in range(4):
            dp = _dot_nt(do, pltpu.bitcast(va32[h, qq], BF16))
            for u in range(QR // DH):
                ringf[dp_at(qq * 16 + u, h, 1)] = dp[0:1, u * DH:(u + 1) * DH]
                ringf[dp_at(qq * 16 + u, H + h, 1)] = dp[1:2, u * DH:(u + 1) * DH]
    lax.fori_loop(0, H, a_dp, None)

    delta = a_delta(0, 2 * H)
    rl = inv[...]

    def a_factors(i, _):
        for r in range(8):
            t = ((i % 2) * 2 + r // 4) * 16 + (i // 2) * 4 + r % 4
            pairs = ring32[i // 2, i % 2, pl.ds(r, H, stride=8), :]
            e = jnp.concatenate([pltpu.bitcast(pairs << 16, F32),
                                 pltpu.bitcast(pairs & jnp.uint32(0xFFFF0000), F32)], axis=0)
            p = e * rl
            ds = p * (ringf[dp_at(t, 0, 2 * H)] - delta) * SCALE
            tile = jnp.concatenate([ds, p], axis=0).T.astype(BF16)
            ring32[12 + t // 16, i // 2, pl.ds((r % 4) * 64, 64), :] = pltpu.bitcast(tile, U32)
    lax.fori_loop(0, 8, a_factors, None)

    def a_grads(grp, lo, stage32, stage, dst, sem):
        def body(i, _):
            q, r = i // 2, (i % 2) * 1024
            for u in range(8):
                sel = select_head(ra, grp * 8 + u, lo)
                for w in range(2):
                    t = pltpu.bitcast(ring32[12 + q, (i % 2) * 2 + w], BF16)
                    rows = pl.ds(_mo((r + w * BR) // 2, BR // 2), BR // 2)
                    stage32(q, u, rows, pltpu.bitcast(_dot(t, sel).astype(BF16), U32))
            for w in range(8):
                rows = pl.ds(_mo(r + w * 128, 128), 128)
                pltpu.make_async_copy(
                    stage(q, rows), dst.at[pl.ds(grp * 8, 8), q, rows], sem).start()
        lax.fori_loop(0, 8, body, None)

    def in_va(h0):
        def put(q, u, rows, val):
            va32[h0 + u, q, rows, :] = val
        return put, lambda q, rows: va.at[pl.ds(h0, 8), q, rows]

    def in_b(buf32, buf):
        def put(q, u, rows, val):
            buf32[q * 8 + u, rows, :] = val
        return put, lambda q, rows: buf.at[pl.ds(q * 8, 8), rows]

    def dva_group(grp, _):
        a_grads(grp, 2 * H, *in_va(grp * 8), dva_h, osem.at[6 + grp])
    lax.fori_loop(0, 4, dva_group, None)

    group = va.at[pl.ds(0, 8)]
    wait_all(kb, osem.at[1])
    a_grads(0, 0, *in_b(kb32, kb), dka_h, osem.at[10])
    wait_all(vb, osem.at[0])
    a_grads(1, 0, *in_b(vb32, vb), dka_h, osem.at[11])

    def dka_group(grp, _):
        wait_all(group, osem.at[4 + grp])
        a_grads(grp, 0, *in_va((grp - 2) * 8), dka_h, osem.at[10 + grp])
    lax.fori_loop(2, 4, dka_group, None)

    out_copy.wait()
    dx_copy.wait()
    wait_all(dkb_h.at[:, pl.ds(0, 3)], zsem.at[0])
    wait_all(dvb_h.at[:, pl.ds(0, 3)], zsem.at[1])
    wait_all(wqb, osem.at[2])
    wait_all(wob, osem.at[3])
    wait_all(wqa, osem.at[4])
    wait_all(woa, osem.at[5])
    for i in range(8, 14):
        wait_all(group, osem.at[i])


@jax.jit
def pallas_interleave_layers__gqa_block_cached__sliding_block_cached__decode_kernel(
    A_x: jax.Array,
    A_k_cache: jax.Array,
    A_v_cache: jax.Array,
    A_wq: jax.Array,
    A_wo: jax.Array,
    B_x: jax.Array,
    B_k_cache: jax.Array,
    B_v_cache: jax.Array,
    B_wq: jax.Array,
    B_wo: jax.Array,
    grad_out: jax.Array,
):
    del B_x
    cache, wq, wo, vec = (H, 4, QR, DH), (D // 128, 128, H * DH), (8, 512, D), (1, 1, D)
    assert A_k_cache.shape == B_k_cache.shape == (1, H, S, DH) and A_x.shape == vec

    hbm = pl.BlockSpec(memory_space=pl.ANY)
    out_shapes = (vec, vec, cache, cache, wq, wo, cache, cache, wq, wo)
    outs = pl.pallas_call(
        _kernel,
        out_shape=[jax.ShapeDtypeStruct(s, BF16) for s in out_shapes],
        in_specs=[hbm] * 10,
        out_specs=[hbm] * 10,
        scratch_shapes=[
            pltpu.VMEM(cache, BF16),
            pltpu.VMEM((H, QR, DH), BF16),
            pltpu.VMEM((H, QR, DH), BF16),
            pltpu.VMEM(wq, BF16),
            pltpu.VMEM(wo, BF16),
            pltpu.VMEM(wq, BF16),
            pltpu.VMEM(wo, BF16),
            pltpu.VMEM((NS, 4, BR, DH), BF16),
            pltpu.VMEM((H, DH, DH), BF16),
            pltpu.VMEM((8, S), F32),
            pltpu.VMEM((4 * H, DH), F32),
            pltpu.VMEM((4 * H, DH), F32),
            pltpu.VMEM((2 * H, DH), F32),
            pltpu.VMEM((2 * H, DH), F32),
            pltpu.VMEM((2 * H, DH), F32),
            pltpu.VMEM((2 * H, DH), F32),
            pltpu.VMEM((2 * H, DH), F32),
            pltpu.VMEM((2 * H, DH), F32),
            pltpu.VMEM((8, 128, DH), BF16),
            pltpu.VMEM(vec, BF16),
            pltpu.VMEM(vec, BF16),
            pltpu.VMEM(vec, BF16),
            pltpu.VMEM(vec, BF16),
            pltpu.SemaphoreType.DMA((NS,)),
            pltpu.SemaphoreType.DMA((8,)),
            pltpu.SemaphoreType.DMA((2, 8)),
            pltpu.SemaphoreType.DMA((4,)),
            pltpu.SemaphoreType.DMA((4,)),
            pltpu.SemaphoreType.DMA((2,)),
            pltpu.SemaphoreType.DMA((14,)),
        ],
        compiler_params=pltpu.CompilerParams(
            vmem_limit_bytes=128 * 1024 * 1024, disable_bounds_checks=True),
    )(A_x, grad_out,
      A_k_cache.reshape(cache), A_v_cache.reshape(cache), A_wq.reshape(wq), A_wo.reshape(wo),
      B_k_cache.reshape(cache), B_v_cache.reshape(cache), B_wq.reshape(wq), B_wo.reshape(wo))
    like = (A_x, A_x, A_k_cache, A_v_cache, A_wq, A_wo, B_k_cache, B_v_cache, B_wq, B_wo)
    return tuple(o.reshape(a.shape) for o, a in zip(outs, like))
```

```python
import jax
from jax import lax
import jax.numpy as jnp
import jax.experimental.pallas as pl
import jax.experimental.pallas.tpu as pltpu
import numpy as np

D = 640
H = 32
DH = 128
QR = 2048
EPS = 1e-5
SCALE = DH ** -0.5

BR = 512
KEEP = 5
FIRST = H - KEEP
J1_SLOT = 4 * KEEP
SPARE_SLOT = J1_SLOT + 2
SLOTS = SPARE_SLOT + 1

DP_SLOT = 4
FA_SLOT = 8
ZERO_SLOT = 16
WB_SLOT = 17
FB_SLOT = 19

ZN = 192

F32 = jnp.float32
BF16 = jnp.bfloat16
U32 = jnp.uint32


def _mo(i, n):
    return i if isinstance(i, int) else pl.multiple_of(i, n)


def _div(i, n):
    if isinstance(i, int):
        return i // n
    return lax.shift_right_logical(i, n.bit_length() - 1) if n & (n - 1) == 0 else lax.div(i, n)


def _rem(i, n):
    if isinstance(i, int):
        return i % n
    return i & (n - 1) if n & (n - 1) == 0 else lax.rem(i, n)


def _at(head):
    return _div(head, 4), _rem(head, 4)


def _dot(a, b):
    return jnp.dot(a, b, preferred_element_type=F32)


def _dot_nt(a, b):
    return lax.dot_general(a, b, (((1,), (1,)), ((), ())), preferred_element_type=F32)


def _iota(shape, axis):
    return lax.broadcasted_iota(jnp.int32, shape, axis)


def _lanes(a):
    return [a[:, u * DH:(u + 1) * DH] for u in range(a.shape[1] // DH)]


def _loop(lo, hi, body, **kwargs):
    lax.fori_loop(lo, hi, lambda i, _: body(i), None, **kwargs)


def _kernel(
        x_h, g_h, ka_h, va_h, wqa_h, woa_h, kb_h, vb_h, wqb_h, wob_h,
        out_h, dx_h, dka_h, dva_h, dwqa_h, dwoa_h, dkb_h, dvb_h, dwqb_h, dwob_h,
        va, kb, vb, wqa, woa, wqb, wob, ring, scores, qa, qb, oa, ob, kbar, vecs,
        zero, x_v, g_v, out_v, dx_v,
        rsem, bsem, wsem, ssem, zsem, osem):
    ring32, ringf = ring.bitcast(U32), ring.bitcast(F32)
    va32, kb32, vb32 = va.bitcast(U32), kb.bitcast(U32), vb.bitcast(U32)
    doa = ringf.at[ZERO_SLOT, 0, pl.ds(128, 2 * H)]
    dob = ringf.at[ZERO_SLOT, 1, pl.ds(128, 2 * H)]
    dq = scores

    def wait_all(buf, sem):
        pltpu.make_async_copy(buf, buf, sem).wait()

    def k_copy(head, c, slot, i):
        src = ka_h.at[(*_at(head), slice(None), pl.ds(_mo(c * BR + i * 32, 32), 32))]
        return pltpu.make_async_copy(
            src, ring.at[slot, :, pl.ds(i * 32, 32), :], rsem.at[slot])

    def k_start(head, c, slot):
        for i in range(BR // 32):
            k_copy(head, c, slot, i).start(priority=i % 2)

    def k_wait(slot):
        wait_all(ring.at[slot], rsem.at[slot])

    def v_copy(grp, q, r):
        sl = (grp, slice(None), q, pl.ds(_mo(r, 32), 32))
        return pltpu.make_async_copy(va_h.at[sl], va.at[sl], rsem.at[SLOTS + grp])

    def b_start(n):
        grp = _div(n, 8)
        for u in range(8):
            r = pl.ds(_mo((_rem(n, 8) * 8 + u) * 32, 32), 32)
            pltpu.make_async_copy(
                kb_h.at[grp, :, 3, r], kb.at[grp, :, r], bsem.at[grp]).start(priority=0)
            pltpu.make_async_copy(
                vb_h.at[grp, :, 3, r], vb.at[grp, :, r], bsem.at[8 + grp]).start(priority=1)

    def wq_start(src, dst, sem, i):
        for u in range(8):
            sl = (slice(None), pl.ds(_mo(i * 8, 8), 8), pl.ds(u * 512, 512))
            pltpu.make_async_copy(src.at[sl], dst.at[sl], sem).start(priority=u % 2)

    def wo_start(src, dst, sem, i):
        for u in range(8):
            sl = (pl.ds((u % 2) * 4, 4), pl.ds(_mo(i * 32 + (u // 2) * 8, 8), 8))
            pltpu.make_async_copy(src.at[sl], dst.at[sl], sem).start(priority=u % 2)

    def zero_start(which, z):
        for half in range(2):
            dst = (dkb_h, dvb_h)[which].at[
                pl.ds(half * 4, 4), _div(z, 48), _rem(_div(z, 16), 3),
                pl.ds(_mo(_rem(z, 16) * 128, 128), 128)]
            src = ring.at[ZERO_SLOT, :, pl.ds(0, 128), :]
            pltpu.make_async_copy(src, dst, zsem.at[which]).start()

    def zero_range(which, lo, hi):
        _loop(lo, hi, lambda z: zero_start(which, z))

    def early_zero_start(z):
        for u in range(8):
            dst = dkb_h.at[pl.ds((u % 2) * 4, 4), _div(z, 48), _rem(_div(z, 16), 3),
                           pl.ds(_mo(_rem(z, 16) * 128 + (u // 2) * 32, 32), 32)]
            pltpu.make_async_copy(zero, dst, zsem.at[0]).start()

    def b_grad_start(src, dst, sem, i):
        grp, r = _div(i, 16), pl.ds(_mo(_rem(i, 16) * 128, 128), 128)
        pltpu.make_async_copy(src.at[:, grp, r], dst.at[:, grp, 3, r], sem).start()

    def dwq_start(src, dst, sem, i):
        sl = (slice(None), pl.ds(_mo(_div(i, 2) * 8, 8), 8),
              pl.ds(_mo(_rem(i, 2) * 2048, 2048), 2048))
        pltpu.make_async_copy(src.at[sl], dst.at[sl], sem).start()

    def dwo_start(src, dst, sem, i):
        sl = (slice(None), pl.ds(_mo(i * 16, 16), 16))
        pltpu.make_async_copy(src.at[sl], dst.at[sl], sem).start()

    def row8(ref, r):
        return jnp.broadcast_to(ref[pl.ds(r, 1), :], (8, ref.shape[1]))

    def pair8(ref, r_even, r_odd):
        return jnp.where(_iota((8, DH), 0) % 2 == 0, row8(ref, r_even), row8(ref, r_odd))

    def four_heads(ref, r):
        return jnp.concatenate([row8(ref, r + u) for u in range(4)], axis=1).astype(BF16)

    def set_four_heads(ref, r, val):
        for u, tile in enumerate(_lanes(val)):
            ref[pl.ds(r + u, 1), :] = tile[0:1]

    def q_proj(n, wq, dst, r):
        n = _lanes(n.astype(BF16))

        def body(i):
            cols = pl.ds(_mo(i * 512, 512), 512)
            set_four_heads(dst, r + 4 * i,
                           sum(_dot(a, wq[k, :, cols]) for k, a in enumerate(n)))
        _loop(0, H // 4, body)

    def q_proj_bwd(src, r, wq):
        def body(i, acc):
            a, cols = four_heads(src, r + 4 * i), pl.ds(_mo(i * 512, 512), 512)
            return acc + jnp.concatenate(
                [_dot_nt(a, wq[k, :, cols]) for k in range(D // 128)], axis=1)
        return lax.fori_loop(0, H // 4, body, jnp.zeros((8, D), F32))

    def o_proj(src, r, wo):
        def body(i, acc):
            return acc + _dot(four_heads(src, r + 4 * i), wo[i])
        return lax.fori_loop(0, H // 4, body, jnp.zeros((8, D), F32))

    def o_proj_bwd(g, wo, dst, r):
        g = g.astype(BF16)
        _loop(0, H // 4, lambda i: set_four_heads(dst, r + 4 * i, _dot_nt(g, wo[i])))

    def set_vec(r, val):
        vecs[pl.ds(r, 1), :] = val[0:1]

    def layernorm(layer):
        x = row8(vecs, 0)
        xc = x - jnp.mean(x, axis=1, keepdims=True)
        sigma = jnp.sqrt(jnp.mean(xc * xc, axis=1, keepdims=True) + EPS)
        n = xc / sigma
        set_vec(layer, n)
        set_vec(4 + layer, jnp.broadcast_to(sigma, (8, D)))
        return n

    def layernorm_bwd(layer, dn):
        n = row8(vecs, layer)
        m1 = jnp.mean(dn, axis=1, keepdims=True)
        m2 = jnp.mean(dn * n, axis=1, keepdims=True)
        return row8(vecs, 8 + layer) + (dn - m1 - n * m2) / row8(vecs, 4 + layer)

    row = _iota((8, DH), 0)
    ninf = jnp.full((8, DH), -jnp.inf, F32)

    def j1_at(head, n=64):
        return (J1_SLOT + _div(head, 16), _rem(_div(head, 4), 4),
                pl.ds(_mo(_rem(head, 4) * 64, 64), n))

    def j3_at(head):
        return (_div(head, 8), 2 + _rem(_div(head, 4), 2),
                pl.ds(_mo(_rem(head, 4) * 64, 64), 64))

    def by_parity(a, reduce, neutral):
        def part(keep):
            b = reduce(jnp.where(keep, a, neutral), axis=0, keepdims=True)
            return reduce(b, axis=1, keepdims=True)
        even = row % 2 == 0
        return jnp.where(even, part(even), part(~even))

    def a_query(head, second):
        return (pair8(qa, head, H + head) if second else row8(qa, head)).astype(BF16)

    def a_scores(q, c, qq, slot, mx):
        tiles = _lanes(_dot_nt(q, pltpu.bitcast(ring32[slot, qq], BF16)))
        s = tiles[0]
        for u in range(1, 4):
            s = jnp.where(row // 2 == u, tiles[u], s)
        s = s * SCALE
        scores[pl.ds(_mo((c * 4 + qq) * 8, 8), 8), :] = s
        return jnp.maximum(mx, s)

    def a_first_scores(head, slot, second):
        q = a_query(head, second)

        def body(c, mx):
            for qq in range(4):
                mx = a_scores(q, c, qq, slot + c, mx)
            return mx
        return by_parity(lax.fori_loop(0, 4, body, ninf), jnp.max, -jnp.inf)

    def a_accumulate(head, c, qq, slot, m, carry):
        acc, ksum, l = carry
        e = jnp.exp(scores[pl.ds((c * 4 + qq) * 8, 8), :] - m)
        e16 = []
        for u in range(4):
            eu = jnp.broadcast_to(e[2 * u + 1:2 * u + 2], (8, DH))
            e16.append(jnp.concatenate([eu, eu], axis=0).astype(BF16))
            k = pltpu.bitcast(ring32[slot, qq, pl.ds(u * 64, 64), :], BF16)
            v = pltpu.bitcast(va32[(*_at(head), qq, pl.ds(c * BR // 2 + u * 64, 64))], BF16)
            w = k.T.astype(F32).reshape(DH // 8, 8, DH) * eu[None]
            w = jnp.concatenate([w.reshape(DH, DH).astype(BF16), e16[u]], axis=0)
            acc = acc + _dot(w, v)
        k = pltpu.bitcast(ring32[slot, qq], BF16)
        ksum = ksum + _dot(jnp.concatenate(e16, axis=1), k)[:8]
        return (acc, ksum, l + e.astype(BF16).astype(F32)), e

    def a_head(head, slots, nxt, nxt_slots, m, second, issue=None, refill=None):
        carry = (jnp.zeros((DH + 16, DH), F32), jnp.zeros((8, DH), F32),
                 jnp.zeros((8, DH), F32))
        q, mx, es = a_query(nxt, second), ninf, []
        for c in range(4):
            for qq in range(4):
                carry, e = a_accumulate(head, c, qq, slots[c], m, carry)
                es.append(e)
                mx = a_scores(q, c, qq, nxt_slots[c], mx)
            pin = pltpu.bitcast(carry[0][:8], U32)
            if refill:
                ring32[refill[c], 0, pl.ds(0, 8), :] = pin
                issue(c)
            elif not second:
                ring32[j1_at(head, 8)] = pin
        acc, ksum, l = carry
        rl = (1.0 / by_parity(l, jnp.sum, 0.0))[1:2]
        out = pl.ds(H + head if second else head, 1)
        oa[out, :] = acc[DH:DH + 1] * rl
        kbar[out, :] = ksum[0:1] * rl
        ring32[(j3_at if second else j1_at)(head)] = pltpu.bitcast(
            (acc[:DH] * rl).astype(BF16), U32)
        if second:
            for i in range(8):
                pairs = jnp.concatenate(es[2 * i:2 * i + 2], axis=0).astype(BF16)
                ring32[i // 2, i % 2, pl.ds(_mo(head * 8, 8), 8), :] = pltpu.bitcast(pairs, U32)
        return by_parity(mx, jnp.max, -jnp.inf)

    def a_delta(r, n):
        do = doa[pl.ds(r, n), :].astype(BF16).astype(F32)
        return jnp.sum(do * oa[pl.ds(r, n), :], axis=1, keepdims=True)

    def a_dq(kpv_at, r):
        def body(head):
            kpv = pltpu.bitcast(ring32[kpv_at(head)], BF16)
            dq[pl.ds(r + head, 1), :] = _dot_nt(row8(doa, r + head).astype(BF16), kpv)[0:1]
        _loop(0, H, body, unroll=4)
        rows = pl.ds(r, H)
        dq[rows, :] = (dq[rows, :] - kbar[rows, :] * a_delta(r, H)) * SCALE

    def b_softmax(q, k):
        s = _dot_nt(q.astype(BF16), k) * SCALE
        e = jnp.exp(s - jnp.max(s, axis=1, keepdims=True))
        return e * (1.0 / jnp.sum(e, axis=1, keepdims=True))

    def b_ds(p, do, v):
        dp = _dot_nt(do.astype(BF16), v)
        return p * (dp - jnp.sum(p * dp, axis=1, keepdims=True)) * SCALE

    def wb_at(t, r, n):
        return (WB_SLOT + _div(t, 8), _rem(_div(t, 2), 4),
                pl.ds(_mo(_rem(t, 2) * 128, 128) + r, n))

    def wb_store(r, val):
        for t, tile in enumerate(_lanes(val)):
            ringf[wb_at(t, r, 1)] = tile

    def select_head(ref, head, values):
        sel = jnp.where(_iota((2 * H, DH), 0) % H == head, ref[...], 0.0).astype(BF16)
        halves = [sel, jnp.zeros_like(sel)]
        return jnp.concatenate(halves[::-1] if values else halves, axis=0)

    def l1_slots(h):
        base = 4 * _rem(h + KEEP - FIRST % KEEP, KEEP)
        return [base, base + 1, base + 2, jnp.where(h == FIRST - 1, SPARE_SLOT, base + 3)]

    def k_prefetch(b):
        k_start(_div(b, 4), _rem(b, 4), l1_slots(_div(b, 4))[0] + _rem(b, 4))

    def v_prefetch(i):
        for u in range(8):
            v_copy(_div(i, 32), _rem(_div(i, 8), 4),
                   _rem(i, 8) * 256 + u * 32).start(priority=u % 2)

    def v_wait(h):
        @pl.when(_rem(h, 4) == 0)
        def _():
            wait_all(va.at[_div(h, 4)], rsem.at[SLOTS + _div(h, 4)])

    x_copy = pltpu.make_async_copy(x_h, x_v, ssem.at[0])
    g_copy = pltpu.make_async_copy(g_h, g_v, ssem.at[1])
    x_copy.start()
    g_copy.start()
    _loop(0, 16, lambda i: wq_start(wqa_h, wqa, wsem.at[0], i))
    _loop(0, 8, k_prefetch)
    zero[...] = jnp.zeros(zero.shape, BF16)
    x_copy.wait()
    g_copy.wait()
    set_vec(0, x_v[0].astype(F32))
    set_vec(12, g_v[0].astype(F32))
    wait_all(wqa, wsem.at[0])
    q_proj(layernorm(1), wqa, qa, 0)
    _loop(0, 8 * KEEP, v_prefetch)
    for slot in l1_slots(0):
        k_wait(slot)
    m = a_first_scores(0, l1_slots(0)[0], False)
    _loop(8, 4 * KEEP, k_prefetch)

    def l1_stream(h, m):
        v_wait(h)
        for slot in l1_slots(h + 1):
            k_wait(slot)
        refill = l1_slots(h + KEEP)

        def issue(c):
            for i in range(BR // 32):
                k_copy(h + KEEP, c, refill[c], i).start(priority=0)
                v_copy(*_at(h + KEEP), c * BR + i * 32).start(priority=1)
        return a_head(h, l1_slots(h), h + 1, l1_slots(h + 1), m, False, issue, refill)
    m = lax.fori_loop(0, FIRST, l1_stream, m)

    _loop(0, 16, lambda i: wo_start(woa_h, woa, wsem.at[1], i))
    _loop(0, 16, lambda i: wq_start(wqb_h, wqb, wsem.at[2], i))

    def l1_tail(h, m):
        v_wait(h)
        nxt = jnp.minimum(h + 1, H - 1)

        @pl.when(h + 1 < H)
        def _():
            for slot in l1_slots(nxt):
                k_wait(slot)
        _loop((h - FIRST) * 4, (h - FIRST + 1) * 4, b_start)
        return a_head(h, l1_slots(h), nxt, l1_slots(nxt), m, False)
    lax.fori_loop(FIRST, H, l1_tail, m)
    _loop(4 * KEEP, 24, b_start)
    wait_all(woa, wsem.at[1])
    set_vec(0, row8(vecs, 0) + o_proj(oa, 0, woa))

    _loop(24, 28, b_start)
    wait_all(wqb, wsem.at[2])
    q_proj(layernorm(2), wqb, qb, 0)

    def l2_head(h):
        @pl.when(_rem(h, 4) == 0)
        def _():
            wait_all(kb.at[_div(h, 4)], bsem.at[_div(h, 4)])
            wait_all(vb.at[_div(h, 4)], bsem.at[8 + _div(h, 4)])

        @pl.when(h < 18)
        def _():
            _loop(28 + 2 * h, 30 + 2 * h, b_start)

        @pl.when((h >= 18) & (h < 22))
        def _():
            _loop((h - 18) * 4, (h - 17) * 4, lambda i: wo_start(wob_h, wob, wsem.at[3], i))

        @pl.when(h >= 27)
        def _():
            for u in range(2):
                early_zero_start((h - 27) * 2 + u)
        p = b_softmax(row8(qb, h), pltpu.bitcast(kb32[_at(h)], BF16))
        ob[pl.ds(h, 1), :] = _dot(p.astype(BF16), pltpu.bitcast(vb32[_at(h)], BF16))[0:1]
    _loop(0, H, l2_head)
    _loop(10, 16, early_zero_start)
    wait_all(wob, wsem.at[3])
    set_vec(0, row8(vecs, 0) + o_proj(ob, 0, wob))

    _loop(16, 20, early_zero_start)
    q_proj(layernorm(3), wqa, qa, H)
    _loop(20, 23, early_zero_start)
    m = a_first_scores(FIRST, 0, True)
    _loop(23, 32, early_zero_start)

    def l3_slots(j):
        base = jnp.where(j == 0, 0, 4 + 4 * _rem(j + KEEP - 2, KEEP - 1))
        return [base, base + 1, base + 2, jnp.where(j == H - 1, SPARE_SLOT, base + 3)]

    def l3_head(j, m, *refill):
        nxt = jnp.minimum(j + 1, H - 1)

        @pl.when((j + 1 >= KEEP) & (j + 1 < H))
        def _():
            for slot in l3_slots(nxt)[:3]:
                k_wait(slot)

        @pl.when((j + 1 >= KEEP) & (j + 1 < H - 1))
        def _():
            k_wait(l3_slots(nxt)[3])
        return a_head(_rem(FIRST + j, H), l3_slots(j), _rem(FIRST + nxt, H), l3_slots(nxt),
                      m, True, *refill)

    def l3_stream(j, m):
        refill = l3_slots(j)

        def issue(c):
            if c % 2:
                for i in range(BR // 32):
                    k_copy(j - 1, c - 1, refill[c - 1], i).start(priority=0)
                    k_copy(j - 1, c, refill[c], i).start(priority=1)
        return l3_head(j, m, issue, refill)

    def l3_quiet(j, m):
        @pl.when(j == FIRST + 1)
        def _():
            _loop(0, 3, lambda c: k_start(FIRST - 1, c, l3_slots(FIRST)[0] + c))

        @pl.when(j == FIRST + 2)
        def _():
            ring32[ZERO_SLOT, :, pl.ds(0, 64), :] = jnp.zeros((4, 64, DH), U32)
            zero_range(0, 32, 60)
        return l3_head(j, m)

    def l3_part(part, m):
        lo = jnp.where(part == 0, 0, FIRST)
        mid = jnp.where(part == 0, 1, H)
        hi = jnp.where(part == 0, FIRST, H)
        return lax.fori_loop(mid, hi, l3_stream, lax.fori_loop(lo, mid, l3_quiet, m))
    lax.fori_loop(0, 2, l3_part, m)
    zero_range(0, 60, 84)
    set_vec(0, row8(vecs, 0) + o_proj(oa, H, woa))

    q_proj(layernorm(4), wqb, qb, H)
    o_proj_bwd(row8(vecs, 12), wob, dob, H)

    def l4_head(h):
        for u in range(3):
            zero_start(0, 84 + 3 * h + u)
        k = pltpu.bitcast(kb32[_at(h)], BF16)
        v = pltpu.bitcast(vb32[_at(h)], BF16)
        p = b_softmax(pair8(qb, h, H + h), k)
        ob[pl.ds(H + h, 1), :] = _dot(p.astype(BF16), v)[1:2]
        ds = b_ds(p, row8(dob, H + h), v)
        dq[pl.ds(3 * H + h, 1), :] = _dot(ds.astype(BF16), k)[1:2]
        wb_store(H + h, ds[1:2])
        wb_store(2 * H + h, p[0:1])
        wb_store(3 * H + h, p[1:2])
    _loop(0, H, l4_head)
    zero_range(0, 84 + 3 * H, ZN)
    zero_range(1, 0, 16)
    out_v[0] = (row8(vecs, 0) + o_proj(ob, H, wob))[0:1].astype(BF16)
    out_copy = pltpu.make_async_copy(out_v, out_h, ssem.at[2])
    out_copy.start()
    set_vec(11, layernorm_bwd(4, q_proj_bwd(dq, 3 * H, wqb)))

    zero_range(1, 16, 32)
    o_proj_bwd(row8(vecs, 11), woa, doa, H)
    a_dq(j3_at, H)
    set_vec(10, layernorm_bwd(3, q_proj_bwd(dq, H, wqa)))

    o_proj_bwd(row8(vecs, 10), wob, dob, 0)

    def l2_bwd_head(h):
        zero_range(1, 32 + h + _div(h, 2), 33 + h + _div(h + 1, 2))
        p = jnp.concatenate(
            [jnp.broadcast_to(ringf[wb_at(t, 2 * H + h, 1)], (8, DH))
             for t in range(QR // DH)], axis=1)
        ds = b_ds(p, row8(dob, h), pltpu.bitcast(vb32[_at(h)], BF16))
        dq[pl.ds(2 * H + h, 1), :] = _dot(
            ds.astype(BF16), pltpu.bitcast(kb32[_at(h)], BF16))[0:1]
        wb_store(h, ds[0:1])
    _loop(0, H, l2_bwd_head)
    zero_range(1, 80, 104)
    set_vec(9, layernorm_bwd(2, q_proj_bwd(dq, 2 * H, wqb)))

    o_proj_bwd(row8(vecs, 9), woa, doa, 0)
    a_dq(j1_at, 0)
    zero_range(1, 104, 120)
    dx_v[0] = layernorm_bwd(1, q_proj_bwd(dq, 0, wqa))[0:1].astype(BF16)
    dx_copy = pltpu.make_async_copy(dx_v, dx_h, ssem.at[3])
    dx_copy.start()

    def b_factors(qq):
        tiles = [ringf[wb_at(qq * 4 + u, 0, 4 * H)].astype(BF16).T for u in range(4)]
        ring32[FB_SLOT, qq] = pltpu.bitcast(jnp.concatenate(tiles, axis=0), U32)
    _loop(0, 4, b_factors)
    zero_range(1, 120, 136)

    def b_grads(grp):
        def body(i):
            u, half = _div(i, 2), _rem(i, 2)
            t = pltpu.bitcast(ring32[FB_SLOT, pl.ds(half * 2, 2)].reshape(BR, DH), BF16)
            for dst, sel in ((vb32, select_head(dob, 4 * u + grp, True)),
                             (kb32, select_head(qb, 4 * u + grp, False))):
                dst[u, grp, pl.ds(_mo(half * BR, BR), BR), :] = pltpu.bitcast(
                    _dot(t, sel).astype(BF16), U32)
        _loop(0, 16, body)
        _loop(grp * 16, (grp + 1) * 16, lambda i: b_grad_start(vb, dvb_h, osem.at[0], i))
        zero_range(1, 136 + grp * 6, 142 + grp * 6)
    _loop(0, 4, b_grads)

    def weight_grads(wq, wo, layer, o, dq_row, sent):
        r = _iota((DH, D), 0)
        n = jnp.where(r == 0, vecs[pl.ds(layer, 1), :],
                      jnp.where(r == 1, vecs[pl.ds(layer + 2, 1), :], 0.0))
        o = jnp.concatenate([o[...], jnp.zeros((2 * H, DH), F32)], axis=0)
        for u, tile in enumerate(_lanes(n) + [o]):
            ring32[DP_SLOT, u // 4, pl.ds((u % 4) * 64, 64), :] = pltpu.bitcast(
                tile.astype(BF16).T, U32)

        def body(head):
            lhs = jnp.concatenate([ring32[DP_SLOT, 0], ring32[DP_SLOT, 1, pl.ds(0, 128), :]])
            lhs = pltpu.bitcast(lhs, BF16)
            sel = jnp.where(r[:, :DH] == 0, dq[pl.ds(dq_row + head, 1), :],
                            jnp.where(r[:, :DH] == 1, dq[pl.ds(dq_row + H + head, 1), :], 0.0))
            dwq = _dot(lhs[:D], sel.astype(BF16)).astype(BF16)
            wq[:, :, pl.ds(_mo(head * DH, DH), DH)] = dwq.reshape(D // DH, DH, DH)
            sel = jnp.where(r == head, vecs[pl.ds(8 + layer, 1), :],
                            jnp.where(r == H + head, vecs[pl.ds(10 + layer, 1), :], 0.0))
            dwo = _dot(lhs[D:], sel.astype(BF16)).astype(BF16)
            wo[_div(head, 4), pl.ds(_mo(_rem(head, 4) * DH, DH), DH), :] = dwo
            b_grad_start(kb, dkb_h, osem.at[1], sent + head)
        _loop(0, H, body)
    weight_grads(wqb, wob, 2, ob, 2 * H, 0)
    weight_grads(wqa, woa, 1, oa, 0, H)

    def dp_at(quarter, t, r, n):
        return (DP_SLOT + quarter, _div(t, 4), pl.ds(_mo(_rem(t, 4) * 64, 64) + r, n))

    def a_dp(h):
        zero_start(1, ZN - H + h)
        dwq_start(wqb, dwqb_h, osem.at[2], h)
        dwo_start(wob, dwob_h, osem.at[3], h)
        dwq_start(wqa, dwqa_h, osem.at[4], h)
        dwo_start(woa, dwoa_h, osem.at[5], h)
        do = pair8(doa, h, H + h).astype(BF16)

        def body(qq):
            dp = _dot_nt(do, pltpu.bitcast(va32[(*_at(h), qq)], BF16))
            for t, tile in enumerate(_lanes(dp)):
                ringf[dp_at(qq, t, h, 1)] = tile[0:1]
                ringf[dp_at(qq, t, H + h, 1)] = tile[1:2]
        _loop(0, 4, body)
    _loop(0, H, a_dp)

    def a_exps(i, r):
        pairs = ring32[_div(i, 2), _rem(i, 2), pl.ds(r, H, stride=8), :]
        return jnp.concatenate([pltpu.bitcast(pairs << 16, F32),
                                pltpu.bitcast(pairs & np.uint32(0xFFFF0000), F32)], axis=0)
    l = lax.fori_loop(0, 8, lambda i, l: l + sum(a_exps(i, r) for r in range(8)),
                      jnp.zeros((2 * H, DH), F32))
    rl = 1.0 / jnp.sum(l, axis=1, keepdims=True)
    delta = a_delta(0, 2 * H)

    def a_factors(i):
        c = _div(i, 2)
        for half in range(2):
            quarter, tiles = _rem(i, 2) * 2 + half, []
            for u in range(4):
                p = a_exps(i, half * 4 + u) * rl
                ds = p * (ringf[dp_at(quarter, c * 4 + u, 0, 2 * H)] - delta) * SCALE
                tiles.append(jnp.concatenate([ds, p], axis=0).astype(BF16).T)
            ring32[FA_SLOT + quarter, c] = pltpu.bitcast(jnp.concatenate(tiles, axis=0), U32)
    _loop(0, 8, a_factors)

    def a_grads(grp, values, stage32, stage, lead, dst, sem):
        def body(i):
            q, half = _div(i, 2), _rem(i, 2)

            def one_head(u):
                sel = select_head(doa if values else qa, 4 * u + grp, values)
                t = ring32[FA_SLOT + q, pl.ds(half * 2, 2)].reshape(BR, DH)
                val = _dot(pltpu.bitcast(t, BF16), sel).astype(BF16)
                stage32[(u, *lead, q, pl.ds(_mo(half * BR, BR), BR))] = pltpu.bitcast(val, U32)
            _loop(0, 8, one_head)

            def send(w):
                rows = pl.ds(_mo(half * 1024 + w * 128, 128), 128)
                pltpu.make_async_copy(stage.at[(slice(None), *lead, q, rows)],
                                      dst.at[:, grp, q, rows], sem).start()
            _loop(0, 8, send)
        _loop(0, 8, body)

    _loop(0, 4, lambda grp: a_grads(grp, True, va32, va, (grp,), dva_h, osem.at[6 + grp]))
    wait_all(dkb_h.at[:, :, 3], osem.at[1])
    a_grads(0, False, kb32, kb, (), dka_h, osem.at[10])
    wait_all(dvb_h.at[:, :, 3], osem.at[0])
    a_grads(1, False, vb32, vb, (), dka_h, osem.at[11])

    def dka_group(grp):
        wait_all(dva_h.at[:, grp - 2], osem.at[4 + grp])
        a_grads(grp, False, va32, va, (grp - 2,), dka_h, osem.at[10 + grp])
    _loop(2, 4, dka_group)

    out_copy.wait()
    dx_copy.wait()
    wait_all(dkb_h.at[:, :, pl.ds(0, 3)], zsem.at[0])
    wait_all(dvb_h.at[:, :, pl.ds(0, 3)], zsem.at[1])
    for i, grad in enumerate((dwqb_h, dwob_h, dwqa_h, dwoa_h)):
        wait_all(grad, osem.at[2 + i])
    for grp in range(2, 4):
        wait_all(dva_h.at[:, grp], osem.at[6 + grp])
    for grp in range(4):
        wait_all(dka_h.at[:, grp], osem.at[10 + grp])


@jax.jit
def pallas_interleave_layers__gqa_block_cached__sliding_block_cached__decode_kernel(
    A_x: jax.Array,
    A_k_cache: jax.Array,
    A_v_cache: jax.Array,
    A_wq: jax.Array,
    A_wo: jax.Array,
    B_x: jax.Array,
    B_k_cache: jax.Array,
    B_v_cache: jax.Array,
    B_wq: jax.Array,
    B_wo: jax.Array,
    grad_out: jax.Array,
):
    del B_x
    cache, window = (H // 4, 4, 4, QR, DH), (H // 4, 4, QR, DH)
    wq, wo, vec = (D // 128, 128, H * DH), (8, 512, D), (1, 1, D)
    assert A_k_cache.shape == B_k_cache.shape == (1, H, 4 * QR, DH) and A_x.shape == vec

    hbm = pl.BlockSpec(memory_space=pl.ANY)
    out_shapes = (vec, vec, cache, cache, wq, wo, cache, cache, wq, wo)
    outs = pl.pallas_call(
        _kernel,
        out_shape=[jax.ShapeDtypeStruct(s, BF16) for s in out_shapes],
        in_specs=[hbm] * 10,
        out_specs=[hbm] * 10,
        scratch_shapes=[
            pltpu.VMEM(cache, BF16),
            pltpu.VMEM(window, BF16),
            pltpu.VMEM(window, BF16),
            pltpu.VMEM(wq, BF16),
            pltpu.VMEM(wo, BF16),
            pltpu.VMEM(wq, BF16),
            pltpu.VMEM(wo, BF16),
            pltpu.VMEM((SLOTS, 4, BR, DH), BF16),
            pltpu.VMEM((4 * H, DH), F32),
            pltpu.VMEM((2 * H, DH), F32),
            pltpu.VMEM((2 * H, DH), F32),
            pltpu.VMEM((2 * H, DH), F32),
            pltpu.VMEM((2 * H, DH), F32),
            pltpu.VMEM((2 * H, DH), F32),
            pltpu.VMEM((16, D), F32),
            pltpu.VMEM((4, 32, DH), BF16),
            pltpu.VMEM(vec, BF16),
            pltpu.VMEM(vec, BF16),
            pltpu.VMEM(vec, BF16),
            pltpu.VMEM(vec, BF16),
            pltpu.SemaphoreType.DMA((SLOTS + 8,)),
            pltpu.SemaphoreType.DMA((16,)),
            pltpu.SemaphoreType.DMA((4,)),
            pltpu.SemaphoreType.DMA((4,)),
            pltpu.SemaphoreType.DMA((2,)),
            pltpu.SemaphoreType.DMA((14,)),
        ],
        compiler_params=pltpu.CompilerParams(
            vmem_limit_bytes=128 * 1024 * 1024, disable_bounds_checks=True),
    )(A_x, grad_out,
      A_k_cache.reshape(cache), A_v_cache.reshape(cache), A_wq.reshape(wq), A_wo.reshape(wo),
      B_k_cache.reshape(cache), B_v_cache.reshape(cache), B_wq.reshape(wq), B_wo.reshape(wo))
    like = (A_x, A_x, A_k_cache, A_v_cache, A_wq, A_wo, B_k_cache, B_v_cache, B_wq, B_wo)
    return tuple(o.reshape(a.shape) for o, a in zip(outs, like))
```

```python
import jax
from jax import lax
import jax.numpy as jnp
import jax.experimental.pallas as pl
import jax.experimental.pallas.tpu as pltpu
import numpy as np

D = 640
H = 32
DH = 128
QR = 2048
EPS = 1e-5
SCALE = DH ** -0.5

BR = 512
KEEP = 5
FIRST = H - KEEP
J1_SLOT = 4 * KEEP
SPARE_SLOT = J1_SLOT + 2
SLOTS = SPARE_SLOT + 1

DP_SLOT = 4
FA_SLOT = 8
ZERO_SLOT = 16
WB_SLOT = 17
FB_SLOT = 19

F32 = jnp.float32
BF16 = jnp.bfloat16
U32 = jnp.uint32


def _mo(i, n):
    return i if isinstance(i, int) else pl.multiple_of(i, n)


def _div(i, n):
    if isinstance(i, int):
        return i // n
    return lax.shift_right_logical(i, n.bit_length() - 1) if n & (n - 1) == 0 else lax.div(i, n)


def _rem(i, n):
    if isinstance(i, int):
        return i % n
    return i & (n - 1) if n & (n - 1) == 0 else lax.rem(i, n)


def _at(head):
    return _div(head, 4), _rem(head, 4)


def _half_at(head, quarter):
    return _div(head, 4), 2 * _rem(head, 4) + _div(quarter, 2), _rem(quarter, 2)


def _dot(a, b):
    return jnp.dot(a, b, preferred_element_type=F32)


def _dot_nt(a, b):
    return lax.dot_general(a, b, (((1,), (1,)), ((), ())), preferred_element_type=F32)


def _iota(shape, axis):
    return lax.broadcasted_iota(jnp.int32, shape, axis)


def _lanes(a):
    return [a[:, u * DH:(u + 1) * DH] for u in range(a.shape[1] // DH)]


def _loop(lo, hi, body, **kwargs):
    lax.fori_loop(lo, hi, lambda i, _: body(i), None, **kwargs)


def _kernel(
        x_h, g_h, ka_h, va_h, wqa_h, woa_h, kb_h, vb_h, wqb_h, wob_h,
        out_h, dx_h, dka_h, dva_h, dwqa_h, dwoa_h, dkb_h, dvb_h, dwqb_h, dwob_h,
        va, kb, vb, wqa, woa, wqb, wob, ring, scores, qa, qb, oa, ob, kbar, vecs,
        zero, x_v, g_v, out_v, dx_v,
        rsem, bsem, wsem, ssem, osem):
    ring32, ringf = ring.bitcast(U32), ring.bitcast(F32)
    va32, kb32, vb32 = va.bitcast(U32), kb.bitcast(U32), vb.bitcast(U32)
    doa = ringf.at[ZERO_SLOT, 0, pl.ds(128, 2 * H)]
    dob = ringf.at[ZERO_SLOT, 1, pl.ds(128, 2 * H)]
    dq = scores

    def wait_all(buf, sem):
        pltpu.make_async_copy(buf, buf, sem).wait()

    def k_copy(head, c, slot, i):
        src = ka_h.at[(*_at(head), slice(None), pl.ds(_mo(c * BR + i * 32, 32), 32))]
        return pltpu.make_async_copy(
            src, ring.at[slot, :, pl.ds(i * 32, 32), :], rsem.at[slot])

    def k_start(head, c, slot):
        for i in range(BR // 32):
            k_copy(head, c, slot, i).start(priority=i % 2)

    def k_wait(slot):
        wait_all(ring.at[slot], rsem.at[slot])

    def v_copy(part, i):
        sl = (_div(part, 4), slice(None), _rem(_div(part, 2), 2),
              pl.ds(_mo(_rem(part, 2) * 1024 + i * 16, 16), 16))
        return pltpu.make_async_copy(va_h.at[sl], va.at[sl], rsem.at[SLOTS + _div(part, 4)])

    def b_start(n):
        grp = _div(n, 8)
        for u in range(8):
            r = pl.ds(_mo((_rem(n, 8) * 8 + u) * 32, 32), 32)
            pltpu.make_async_copy(
                kb_h.at[grp, :, 3, r], kb.at[grp, :, r], bsem.at[grp]).start(priority=0)
            pltpu.make_async_copy(
                vb_h.at[grp, :, 3, r], vb.at[grp, :, r], bsem.at[8 + grp]).start(priority=1)

    def wq_start(src, dst, sem, i):
        for u in range(8):
            sl = (slice(None), pl.ds(_mo(i * 8, 8), 8), pl.ds(u * 512, 512))
            pltpu.make_async_copy(src.at[sl], dst.at[sl], sem).start(priority=u % 2)

    def wo_start(src, dst, sem, i):
        for u in range(8):
            sl = (pl.ds((u % 2) * 4, 4), pl.ds(_mo(i * 32 + (u // 2) * 8, 8), 8))
            pltpu.make_async_copy(src.at[sl], dst.at[sl], sem).start(priority=u % 2)

    def zero_start(which, z):
        for half in range(2):
            dst = (dkb_h, dvb_h)[which].at[
                _div(z, 16), pl.ds(half * 4, 4), 0, pl.ds(_mo(_rem(z, 16) * 128, 128), 128)]
            src = ring.at[ZERO_SLOT, :, pl.ds(0, 128), :]
            pltpu.make_async_copy(src, dst, osem.at[which]).start()

    def zero_range(which, lo, hi):
        _loop(lo, hi, lambda z: zero_start(which, z))

    def small_zero_start(which, z):
        for u in range(8):
            dst = (dkb_h, dvb_h)[which].at[
                :, 2 * _div(z, 16), 1, pl.ds(_mo(_rem(z, 16) * 128 + u * 16, 16), 16)]
            pltpu.make_async_copy(zero, dst, osem.at[which]).start()

    def b_grad_start(which, z):
        b, rows = _div(z, 16), pl.ds(_mo(_rem(z, 16) * 128, 128), 128)
        pltpu.make_async_copy((kb, vb)[which].at[:, b, rows],
                              (dkb_h, dvb_h)[which].at[:, 2 * b + 1, 1, rows],
                              osem.at[which]).start()

    def dwq_start(src, dst, sem, i):
        sl = (slice(None), pl.ds(_mo(_div(i, 2) * 8, 8), 8),
              pl.ds(_mo(_rem(i, 2) * 2048, 2048), 2048))
        pltpu.make_async_copy(src.at[sl], dst.at[sl], sem).start()

    def dwo_start(src, dst, sem, i):
        sl = (slice(None), pl.ds(_mo(i * 16, 16), 16))
        pltpu.make_async_copy(src.at[sl], dst.at[sl], sem).start()

    def row8(ref, r):
        return jnp.broadcast_to(ref[pl.ds(r, 1), :], (8, ref.shape[1]))

    def pair8(ref, r_even, r_odd):
        return jnp.where(_iota((8, DH), 0) % 2 == 0, row8(ref, r_even), row8(ref, r_odd))

    def four_heads(ref, r):
        return jnp.concatenate([row8(ref, r + u) for u in range(4)], axis=1).astype(BF16)

    def set_four_heads(ref, r, val):
        for u, tile in enumerate(_lanes(val)):
            ref[pl.ds(r + u, 1), :] = tile[0:1]

    def q_proj(n, wq, dst, r):
        n = _lanes(n.astype(BF16))

        def body(i):
            cols = pl.ds(_mo(i * 512, 512), 512)
            set_four_heads(dst, r + 4 * i,
                           sum(_dot(a, wq[k, :, cols]) for k, a in enumerate(n)))
        _loop(0, H // 4, body)

    def q_proj_bwd(src, r, wq):
        def body(i, acc):
            a, cols = four_heads(src, r + 4 * i), pl.ds(_mo(i * 512, 512), 512)
            return acc + jnp.concatenate(
                [_dot_nt(a, wq[k, :, cols]) for k in range(D // 128)], axis=1)
        return lax.fori_loop(0, H // 4, body, jnp.zeros((8, D), F32))

    def o_proj(src, r, wo):
        def body(i, acc):
            return acc + _dot(four_heads(src, r + 4 * i), wo[i])
        return lax.fori_loop(0, H // 4, body, jnp.zeros((8, D), F32))

    def o_proj_bwd(g, wo, dst, r):
        g = g.astype(BF16)
        _loop(0, H // 4, lambda i: set_four_heads(dst, r + 4 * i, _dot_nt(g, wo[i])))

    def set_vec(r, val):
        vecs[pl.ds(r, 1), :] = val[0:1]

    def layernorm(layer):
        x = row8(vecs, 0)
        xc = x - jnp.mean(x, axis=1, keepdims=True)
        sigma = jnp.sqrt(jnp.mean(xc * xc, axis=1, keepdims=True) + EPS)
        n = xc / sigma
        set_vec(layer, n)
        set_vec(4 + layer, jnp.broadcast_to(sigma, (8, D)))
        return n

    def layernorm_bwd(layer, dn):
        n = row8(vecs, layer)
        m1 = jnp.mean(dn, axis=1, keepdims=True)
        m2 = jnp.mean(dn * n, axis=1, keepdims=True)
        return row8(vecs, 8 + layer) + (dn - m1 - n * m2) / row8(vecs, 4 + layer)

    row = _iota((8, DH), 0)
    ninf = jnp.full((8, DH), -jnp.inf, F32)

    def j1_at(head, n=64):
        return (J1_SLOT + _div(head, 16), _rem(_div(head, 4), 4),
                pl.ds(_mo(_rem(head, 4) * 64, 64), n))

    def j3_at(head):
        return (_div(head, 8), 2 + _rem(_div(head, 4), 2),
                pl.ds(_mo(_rem(head, 4) * 64, 64), 64))

    def by_parity(a, reduce, neutral):
        def part(keep):
            b = reduce(jnp.where(keep, a, neutral), axis=0, keepdims=True)
            return reduce(b, axis=1, keepdims=True)
        even = row % 2 == 0
        return jnp.where(even, part(even), part(~even))

    def a_query(head, second):
        return (pair8(qa, head, H + head) if second else row8(qa, head)).astype(BF16)

    def a_scores(q, c, qq, slot, mx):
        tiles = _lanes(_dot_nt(q, pltpu.bitcast(ring32[slot, qq], BF16)))
        s = tiles[0]
        for u in range(1, 4):
            s = jnp.where(row // 2 == u, tiles[u], s)
        s = s * SCALE
        scores[pl.ds(_mo((c * 4 + qq) * 8, 8), 8), :] = s
        return jnp.maximum(mx, s)

    def a_first_scores(head, slot, second):
        q = a_query(head, second)

        def body(c, mx):
            for qq in range(4):
                mx = a_scores(q, c, qq, slot + c, mx)
            return mx
        return by_parity(lax.fori_loop(0, 4, body, ninf), jnp.max, -jnp.inf)

    def a_accumulate(head, c, qq, slot, m, carry):
        acc, ksum, l = carry
        e = jnp.exp(scores[pl.ds((c * 4 + qq) * 8, 8), :] - m)
        e16 = []
        for u in range(4):
            eu = jnp.broadcast_to(e[2 * u + 1:2 * u + 2], (8, DH))
            e16.append(jnp.concatenate([eu, eu], axis=0).astype(BF16))
            k = pltpu.bitcast(ring32[slot, qq, pl.ds(u * 64, 64), :], BF16)
            v = pltpu.bitcast(va32[(*_half_at(head, qq), pl.ds(c * BR // 2 + u * 64, 64))], BF16)
            w = k.T.astype(F32).reshape(DH // 8, 8, DH) * eu[None]
            w = jnp.concatenate([w.reshape(DH, DH).astype(BF16), e16[u]], axis=0)
            acc = acc + _dot(w, v)
        k = pltpu.bitcast(ring32[slot, qq], BF16)
        ksum = ksum + _dot(jnp.concatenate(e16, axis=1), k)[:8]
        return (acc, ksum, l + e.astype(BF16).astype(F32)), e

    def a_head(head, slots, nxt, nxt_slots, m, second, issue=None, refill=None):
        carry = (jnp.zeros((DH + 16, DH), F32), jnp.zeros((8, DH), F32),
                 jnp.zeros((8, DH), F32))
        q, mx, es = a_query(nxt, second), ninf, []
        for c in range(4):
            for qq in range(4):
                carry, e = a_accumulate(head, c, qq, slots[c], m, carry)
                es.append(e)
                mx = a_scores(q, c, qq, nxt_slots[c], mx)
            pin = pltpu.bitcast(carry[0][:8], U32)
            if refill:
                ring32[refill[c], 0, pl.ds(0, 8), :] = pin
                issue(c)
            elif not second:
                ring32[j1_at(head, 8)] = pin
        acc, ksum, l = carry
        rl = (1.0 / by_parity(l, jnp.sum, 0.0))[1:2]
        out = pl.ds(H + head if second else head, 1)
        oa[out, :] = acc[DH:DH + 1] * rl
        kbar[out, :] = ksum[0:1] * rl
        ring32[(j3_at if second else j1_at)(head)] = pltpu.bitcast(
            (acc[:DH] * rl).astype(BF16), U32)
        if second:
            for i in range(8):
                pairs = jnp.concatenate(es[2 * i:2 * i + 2], axis=0).astype(BF16)
                ring32[i // 2, i % 2, pl.ds(_mo(head * 8, 8), 8), :] = pltpu.bitcast(pairs, U32)
        return by_parity(mx, jnp.max, -jnp.inf)

    def a_delta(r, n):
        do = doa[pl.ds(r, n), :].astype(BF16).astype(F32)
        return jnp.sum(do * oa[pl.ds(r, n), :], axis=1, keepdims=True)

    def a_dq(kpv_at, r):
        def body(head):
            kpv = pltpu.bitcast(ring32[kpv_at(head)], BF16)
            dq[pl.ds(r + head, 1), :] = _dot_nt(row8(doa, r + head).astype(BF16), kpv)[0:1]
        _loop(0, H, body, unroll=4)
        rows = pl.ds(r, H)
        dq[rows, :] = (dq[rows, :] - kbar[rows, :] * a_delta(r, H)) * SCALE

    def b_softmax(q, k):
        s = _dot_nt(q.astype(BF16), k) * SCALE
        e = jnp.exp(s - jnp.max(s, axis=1, keepdims=True))
        return e * (1.0 / jnp.sum(e, axis=1, keepdims=True))

    def b_ds(p, do, v):
        dp = _dot_nt(do.astype(BF16), v)
        return p * (dp - jnp.sum(p * dp, axis=1, keepdims=True)) * SCALE

    def wb_at(t, r, n):
        return (WB_SLOT + _div(t, 8), _rem(_div(t, 2), 4),
                pl.ds(_mo(_rem(t, 2) * 128, 128) + r, n))

    def wb_store(r, val):
        for t, tile in enumerate(_lanes(val)):
            ringf[wb_at(t, r, 1)] = tile

    def select_head(ref, head, values):
        sel = jnp.where(_iota((2 * H, DH), 0) % H == head, ref[...], 0.0).astype(BF16)
        halves = [sel, jnp.zeros_like(sel)]
        return jnp.concatenate(halves[::-1] if values else halves, axis=0)

    def l1_slots(h):
        base = 4 * _rem(h + KEEP - FIRST % KEEP, KEEP)
        return [base, base + 1, base + 2, jnp.where(h == FIRST - 1, SPARE_SLOT, base + 3)]

    def k_prefetch(b):
        k_start(_div(b, 4), _rem(b, 4), l1_slots(_div(b, 4))[0] + _rem(b, 4))

    def v_prefetch(i):
        for u in range(8):
            v_copy(_div(i, 8), _rem(i, 8) * 8 + u).start(priority=u % 2)

    def v_wait(h):
        @pl.when(_rem(h, 4) == 0)
        def _():
            wait_all(va.at[_div(h, 4)], rsem.at[SLOTS + _div(h, 4)])

    x_copy = pltpu.make_async_copy(x_h, x_v, ssem.at[0])
    g_copy = pltpu.make_async_copy(g_h, g_v, ssem.at[1])
    x_copy.start()
    g_copy.start()
    _loop(0, 16, lambda i: wq_start(wqa_h, wqa, wsem.at[0], i))
    _loop(0, 8, k_prefetch)
    zero[...] = jnp.zeros(zero.shape, BF16)
    x_copy.wait()
    g_copy.wait()
    set_vec(0, x_v[0].astype(F32))
    set_vec(12, g_v[0].astype(F32))
    wait_all(wqa, wsem.at[0])
    q_proj(layernorm(1), wqa, qa, 0)
    _loop(0, 8 * KEEP, v_prefetch)
    for slot in l1_slots(0):
        k_wait(slot)
    m = a_first_scores(0, l1_slots(0)[0], False)
    _loop(8, 4 * KEEP, k_prefetch)

    def l1_stream(h, m):
        v_wait(h)
        for slot in l1_slots(h + 1):
            k_wait(slot)
        refill = l1_slots(h + KEEP)

        def issue(c):
            for i in range(BR // 32):
                k_copy(h + KEEP, c, refill[c], i).start(priority=0)
                v_copy(h + KEEP, c * 16 + i).start(priority=1)
        return a_head(h, l1_slots(h), h + 1, l1_slots(h + 1), m, False, issue, refill)
    m = lax.fori_loop(0, FIRST, l1_stream, m)

    _loop(0, 16, lambda i: wo_start(woa_h, woa, wsem.at[1], i))
    _loop(0, 16, lambda i: wq_start(wqb_h, wqb, wsem.at[2], i))

    def l1_tail(h, m):
        v_wait(h)
        nxt = jnp.minimum(h + 1, H - 1)

        @pl.when(h + 1 < H)
        def _():
            for slot in l1_slots(nxt):
                k_wait(slot)
        _loop((h - FIRST) * 4, (h - FIRST + 1) * 4, b_start)
        return a_head(h, l1_slots(h), nxt, l1_slots(nxt), m, False)
    lax.fori_loop(FIRST, H, l1_tail, m)
    _loop(4 * KEEP, 24, b_start)
    wait_all(woa, wsem.at[1])
    set_vec(0, row8(vecs, 0) + o_proj(oa, 0, woa))

    _loop(24, 28, b_start)
    wait_all(wqb, wsem.at[2])
    q_proj(layernorm(2), wqb, qb, 0)

    def l2_head(h):
        @pl.when(_rem(h, 4) == 0)
        def _():
            wait_all(kb.at[_div(h, 4)], bsem.at[_div(h, 4)])
            wait_all(vb.at[_div(h, 4)], bsem.at[8 + _div(h, 4)])

        @pl.when(h < 18)
        def _():
            _loop(28 + 2 * h, 30 + 2 * h, b_start)

        @pl.when((h >= 18) & (h < 22))
        def _():
            _loop((h - 18) * 4, (h - 17) * 4, lambda i: wo_start(wob_h, wob, wsem.at[3], i))

        @pl.when(h >= 27)
        def _():
            for u in range(2):
                small_zero_start(0, (h - 27) * 2 + u)
        p = b_softmax(row8(qb, h), pltpu.bitcast(kb32[_at(h)], BF16))
        ob[pl.ds(h, 1), :] = _dot(p.astype(BF16), pltpu.bitcast(vb32[_at(h)], BF16))[0:1]
    _loop(0, H, l2_head)
    _loop(10, 17, lambda z: small_zero_start(0, z))
    wait_all(wob, wsem.at[3])
    set_vec(0, row8(vecs, 0) + o_proj(ob, 0, wob))

    _loop(17, 22, lambda z: small_zero_start(0, z))
    q_proj(layernorm(3), wqa, qa, H)
    _loop(22, 25, lambda z: small_zero_start(0, z))
    m = a_first_scores(FIRST, 0, True)
    _loop(25, 34, lambda z: small_zero_start(0, z))

    def l3_slots(j):
        odd, lap = _rem(j + 1, 2), _rem(_div(j + 3, 4) + 1, 2)
        base = 4 + 8 * _rem(_div(j + 3, 2), 2)
        slots = []
        for c in range(4):
            slot = base + jnp.where(lap == 0, 4 * odd + c, 4 * (c // 2) + 2 * odd + c % 2)
            last = (12, 13, 14, SPARE_SLOT)[c]
            slots.append(jnp.where(j == 0, c, jnp.where(j == H - 1, last, slot)))
        return slots

    def l3_head(j, m, *refill):
        nxt = jnp.minimum(j + 1, H - 1)

        @pl.when((j + 1 >= KEEP) & (j + 1 < H))
        def _():
            for slot in l3_slots(nxt)[:3]:
                k_wait(slot)

        @pl.when((j + 1 >= KEEP) & (j + 1 < H - 1))
        def _():
            k_wait(l3_slots(nxt)[3])
        return a_head(_rem(FIRST + j, H), l3_slots(j), _rem(FIRST + nxt, H), l3_slots(nxt),
                      m, True, *refill)

    def l3_stream(j, m):
        refill = l3_slots(j)

        def issue(c):
            if c >= 2:
                head, block = (j - 1) & ~1, _rem(j - 1, 2) * 2 + c - 2
                for i in range(BR // 32):
                    k_copy(head, block, refill[c - 2], i).start(priority=0)
                    k_copy(head + 1, block, refill[c], i).start(priority=1)
        return l3_head(j, m, issue, refill)

    def l3_quiet(j, m):
        @pl.when(j == FIRST + 1)
        def _():
            _loop(0, 3, lambda c: k_start(FIRST - 1, c, 12 + c))

        @pl.when(j == FIRST + 2)
        def _():
            ring32[ZERO_SLOT, :, pl.ds(0, 64), :] = jnp.zeros((4, 64, DH), U32)
            zero_range(0, 0, 28)
        return l3_head(j, m)

    def l3_part(part, m):
        lo = jnp.where(part == 0, 0, FIRST)
        mid = jnp.where(part == 0, 1, H)
        hi = jnp.where(part == 0, FIRST, H)
        return lax.fori_loop(mid, hi, l3_stream, lax.fori_loop(lo, mid, l3_quiet, m))
    lax.fori_loop(0, 2, l3_part, m)
    zero_range(0, 28, 52)
    set_vec(0, row8(vecs, 0) + o_proj(oa, H, woa))

    q_proj(layernorm(4), wqb, qb, H)
    o_proj_bwd(row8(vecs, 12), wob, dob, H)

    def l4_head(h):
        @pl.when(h < 10)
        def _():
            for u in range(3):
                small_zero_start(0, 34 + 3 * h + u)

        @pl.when((h >= 10) & (h < H - 1))
        def _():
            for u in range(3):
                small_zero_start(1, 3 * (h - 10) + u)
        k = pltpu.bitcast(kb32[_at(h)], BF16)
        v = pltpu.bitcast(vb32[_at(h)], BF16)
        p = b_softmax(pair8(qb, h, H + h), k)
        ob[pl.ds(H + h, 1), :] = _dot(p.astype(BF16), v)[1:2]
        ds = b_ds(p, row8(dob, H + h), v)
        dq[pl.ds(3 * H + h, 1), :] = _dot(ds.astype(BF16), k)[1:2]
        wb_store(H + h, ds[1:2])
        wb_store(2 * H + h, p[0:1])
        wb_store(3 * H + h, p[1:2])
    _loop(0, H, l4_head)
    small_zero_start(1, 63)
    zero_range(0, 52, 80)
    out_v[0] = (row8(vecs, 0) + o_proj(ob, H, wob))[0:1].astype(BF16)
    out_copy = pltpu.make_async_copy(out_v, out_h, ssem.at[2])
    out_copy.start()
    set_vec(11, layernorm_bwd(4, q_proj_bwd(dq, 3 * H, wqb)))

    zero_range(0, 80, 96)
    o_proj_bwd(row8(vecs, 11), woa, doa, H)
    a_dq(j3_at, H)
    set_vec(10, layernorm_bwd(3, q_proj_bwd(dq, H, wqa)))

    o_proj_bwd(row8(vecs, 10), wob, dob, 0)

    def l2_bwd_head(h):
        zero_range(1, h + _div(h, 2), 1 + h + _div(h + 1, 2))
        p = jnp.concatenate(
            [jnp.broadcast_to(ringf[wb_at(t, 2 * H + h, 1)], (8, DH))
             for t in range(QR // DH)], axis=1)
        ds = b_ds(p, row8(dob, h), pltpu.bitcast(vb32[_at(h)], BF16))
        dq[pl.ds(2 * H + h, 1), :] = _dot(
            ds.astype(BF16), pltpu.bitcast(kb32[_at(h)], BF16))[0:1]
        wb_store(h, ds[0:1])
    _loop(0, H, l2_bwd_head)
    zero_range(0, 96, 120)
    set_vec(9, layernorm_bwd(2, q_proj_bwd(dq, 2 * H, wqb)))

    o_proj_bwd(row8(vecs, 9), woa, doa, 0)
    a_dq(j1_at, 0)
    zero_range(0, 120, 128)
    zero_range(1, 48, 56)
    dx_v[0] = layernorm_bwd(1, q_proj_bwd(dq, 0, wqa))[0:1].astype(BF16)
    dx_copy = pltpu.make_async_copy(dx_v, dx_h, ssem.at[3])
    dx_copy.start()

    def b_factors(qq):
        tiles = [ringf[wb_at(qq * 4 + u, 0, 4 * H)].astype(BF16).T for u in range(4)]
        ring32[FB_SLOT, qq] = pltpu.bitcast(jnp.concatenate(tiles, axis=0), U32)
    _loop(0, 4, b_factors)
    zero_range(1, 56, 64)

    def b_grads(which, stage32, vectors):
        def group(b):
            def body(i):
                a, half = _div(i, 2), _rem(i, 2)
                t = ring32[FB_SLOT, pl.ds(half * 2, 2)].reshape(BR, DH)
                val = _dot(pltpu.bitcast(t, BF16), select_head(vectors, 4 * a + b, which == 1))
                stage32[a, b, pl.ds(_mo(half * BR, BR), BR), :] = pltpu.bitcast(
                    val.astype(BF16), U32)
            _loop(0, 16, body)
            _loop(b * 16, (b + 1) * 16, lambda z: b_grad_start(which, z))
        _loop(0, 4, group)
    b_grads(1, vb32, dob)
    b_grads(0, kb32, qb)

    def weight_grads(wq, wo, layer, o, dq_row, z0):
        r = _iota((DH, D), 0)
        n = jnp.where(r == 0, vecs[pl.ds(layer, 1), :],
                      jnp.where(r == 1, vecs[pl.ds(layer + 2, 1), :], 0.0))
        o = jnp.concatenate([o[...], jnp.zeros((2 * H, DH), F32)], axis=0)
        for u, tile in enumerate(_lanes(n) + [o]):
            ring32[DP_SLOT, u // 4, pl.ds((u % 4) * 64, 64), :] = pltpu.bitcast(
                tile.astype(BF16).T, U32)

        def body(head):
            lhs = jnp.concatenate([ring32[DP_SLOT, 0], ring32[DP_SLOT, 1, pl.ds(0, 128), :]])
            lhs = pltpu.bitcast(lhs, BF16)
            sel = jnp.where(r[:, :DH] == 0, dq[pl.ds(dq_row + head, 1), :],
                            jnp.where(r[:, :DH] == 1, dq[pl.ds(dq_row + H + head, 1), :], 0.0))
            dwq = _dot(lhs[:D], sel.astype(BF16)).astype(BF16)
            wq[:, :, pl.ds(_mo(head * DH, DH), DH)] = dwq.reshape(D // DH, DH, DH)
            sel = jnp.where(r == head, vecs[pl.ds(8 + layer, 1), :],
                            jnp.where(r == H + head, vecs[pl.ds(10 + layer, 1), :], 0.0))
            dwo = _dot(lhs[D:], sel.astype(BF16)).astype(BF16)
            wo[_div(head, 4), pl.ds(_mo(_rem(head, 4) * DH, DH), DH), :] = dwo
            zero_start(1, z0 + head)
        _loop(0, H, body)
    weight_grads(wqb, wob, 2, ob, 2 * H, 64)
    weight_grads(wqa, woa, 1, oa, 0, 96)

    def dp_at(quarter, t, r, n):
        return (DP_SLOT + quarter, _div(t, 4), pl.ds(_mo(_rem(t, 4) * 64, 64) + r, n))

    weight_grad_copies = ((dwq_start, wqb, dwqb_h), (dwo_start, wob, dwob_h),
                          (dwq_start, wqa, dwqa_h), (dwo_start, woa, dwoa_h))

    def a_dp(h):
        for i, (start, src, dst) in enumerate(weight_grad_copies):
            @pl.when(_div(h, 8) == i)
            def _():
                for u in range(4):
                    start(src, dst, osem.at[2 + i], _rem(h, 8) * 4 + u)
        do = pair8(doa, h, H + h).astype(BF16)

        def body(qq):
            dp = _dot_nt(do, pltpu.bitcast(va32[_half_at(h, qq)], BF16))
            for t, tile in enumerate(_lanes(dp)):
                ringf[dp_at(qq, t, h, 1)] = tile[0:1]
                ringf[dp_at(qq, t, H + h, 1)] = tile[1:2]
        _loop(0, 4, body, unroll=True)
    _loop(0, H, a_dp)

    def a_exps(i, r):
        pairs = ring32[_div(i, 2), _rem(i, 2), pl.ds(r, H, stride=8), :]
        return jnp.concatenate([pltpu.bitcast(pairs << 16, F32),
                                pltpu.bitcast(pairs & np.uint32(0xFFFF0000), F32)], axis=0)
    l = lax.fori_loop(0, 8, lambda i, l: l + sum(a_exps(i, r) for r in range(8)),
                      jnp.zeros((2 * H, DH), F32))
    rl = 1.0 / jnp.sum(l, axis=1, keepdims=True)
    delta = a_delta(0, 2 * H)

    def a_factors(i):
        c = _div(i, 2)
        for half in range(2):
            quarter, tiles = _rem(i, 2) * 2 + half, []
            for u in range(4):
                p = a_exps(i, half * 4 + u) * rl
                ds = p * (ringf[dp_at(quarter, c * 4 + u, 0, 2 * H)] - delta) * SCALE
                tiles.append(jnp.concatenate([ds, p], axis=0).astype(BF16).T)
            ring32[FA_SLOT + quarter, c] = pltpu.bitcast(jnp.concatenate(tiles, axis=0), U32)
    _loop(0, 8, a_factors)

    def a_grads(a, values, stage32, stage, place, dst, sem):
        def body(i):
            q, half = _div(i, 2), _rem(i, 2)

            def one_block(u):
                sel = select_head(doa if values else qa, 4 * a + _div(u, 2), values)
                t = ring32[FA_SLOT + 2 * _rem(u, 2) + q, pl.ds(half * 2, 2)].reshape(BR, DH)
                val = _dot(pltpu.bitcast(t, BF16), sel).astype(BF16)
                stage32[(*place(u, q), pl.ds(_mo(half * BR, BR), BR))] = pltpu.bitcast(val, U32)
            _loop(0, 8, one_block)

            def send(w):
                for u in range(8):
                    rows = pl.ds(_mo(half * 1024 + w * 128 + u * 16, 16), 16)
                    pltpu.make_async_copy(stage.at[(*place(slice(None), q), rows)],
                                          dst.at[a, :, q, rows], sem).start()
            _loop(0, 8, send)
        _loop(0, 4, body)

    _loop(0, 8, lambda a: a_grads(a, True, va32, va, lambda u, q: (a, u, q),
                                  dva_h, osem.at[7 + a]))
    for which, (stage32, stage) in enumerate(((kb32, kb), (vb32, vb))):
        wait_all((dkb_h, dvb_h)[which], osem.at[which])
        _loop(0, 2, lambda a: a_grads(2 * which + a, False, stage32, stage,
                                      lambda u, q: (u, 2 * a + q), dka_h, osem.at[6]))

    def dka_rest(a):
        wait_all(dva_h.at[a - 4], osem.at[3 + a])
        a_grads(a, False, va32, va, lambda u, q: (a - 4, u, q), dka_h, osem.at[6])
    _loop(4, 8, dka_rest)

    out_copy.wait()
    dx_copy.wait()
    for i, (_, _, dst) in enumerate(weight_grad_copies):
        wait_all(dst, osem.at[2 + i])
    for a in range(4, 8):
        wait_all(dva_h.at[a], osem.at[7 + a])
    wait_all(dka_h, osem.at[6])


@jax.jit
def pallas_interleave_layers__gqa_block_cached__sliding_block_cached__decode_kernel(
    A_x: jax.Array,
    A_k_cache: jax.Array,
    A_v_cache: jax.Array,
    A_wq: jax.Array,
    A_wo: jax.Array,
    B_x: jax.Array,
    B_k_cache: jax.Array,
    B_v_cache: jax.Array,
    B_wq: jax.Array,
    B_wo: jax.Array,
    grad_out: jax.Array,
):
    del B_x
    cache, halves, window = (H // 4, 4, 4, QR, DH), (H // 4, 8, 2, QR, DH), (H // 4, 4, QR, DH)
    wq, wo, vec = (D // 128, 128, H * DH), (8, 512, D), (1, 1, D)
    assert A_k_cache.shape == B_k_cache.shape == (1, H, 4 * QR, DH) and A_x.shape == vec

    hbm = pl.BlockSpec(memory_space=pl.ANY)
    out_shapes = (vec, vec, halves, halves, wq, wo, halves, halves, wq, wo)
    outs = pl.pallas_call(
        _kernel,
        out_shape=[jax.ShapeDtypeStruct(s, BF16) for s in out_shapes],
        in_specs=[hbm] * 10,
        out_specs=[hbm] * 10,
        scratch_shapes=[
            pltpu.VMEM(halves, BF16),
            pltpu.VMEM(window, BF16),
            pltpu.VMEM(window, BF16),
            pltpu.VMEM(wq, BF16),
            pltpu.VMEM(wo, BF16),
            pltpu.VMEM(wq, BF16),
            pltpu.VMEM(wo, BF16),
            pltpu.VMEM((SLOTS, 4, BR, DH), BF16),
            pltpu.VMEM((4 * H, DH), F32),
            pltpu.VMEM((2 * H, DH), F32),
            pltpu.VMEM((2 * H, DH), F32),
            pltpu.VMEM((2 * H, DH), F32),
            pltpu.VMEM((2 * H, DH), F32),
            pltpu.VMEM((2 * H, DH), F32),
            pltpu.VMEM((16, D), F32),
            pltpu.VMEM((8, 16, DH), BF16),
            pltpu.VMEM(vec, BF16),
            pltpu.VMEM(vec, BF16),
            pltpu.VMEM(vec, BF16),
            pltpu.VMEM(vec, BF16),
            pltpu.SemaphoreType.DMA((SLOTS + 8,)),
            pltpu.SemaphoreType.DMA((16,)),
            pltpu.SemaphoreType.DMA((4,)),
            pltpu.SemaphoreType.DMA((4,)),
            pltpu.SemaphoreType.DMA((15,)),
        ],
        compiler_params=pltpu.CompilerParams(
            vmem_limit_bytes=128 * 1024 * 1024, disable_bounds_checks=True),
    )(A_x, grad_out,
      A_k_cache.reshape(cache), A_v_cache.reshape(halves), A_wq.reshape(wq), A_wo.reshape(wo),
      B_k_cache.reshape(cache), B_v_cache.reshape(cache), B_wq.reshape(wq), B_wo.reshape(wo))
    like = (A_x, A_x, A_k_cache, A_v_cache, A_wq, A_wo, B_k_cache, B_v_cache, B_wq, B_wo)
    return tuple(o.reshape(a.shape) for o, a in zip(outs, like))
```
